```python
import jax
import jax.numpy as jnp

def _softmax(x, axis=-1):
    return jax.nn.softmax(x, axis=axis)

def _gelu(x):
    return jax.nn.gelu(x, approximate=True)

def _silu(x):
    return jax.nn.silu(x)

def _sigmoid(x):
    return jax.nn.sigmoid(x)

def _layernorm(x, axis=-1, eps=1e-05):
    m = jnp.mean(x, axis=axis, keepdims=True)
    v = jnp.var(x, axis=axis, keepdims=True)
    return (x - m) / jnp.sqrt(v + eps)

def _scatter_add(tgt, idx, src, axis=0):
    return tgt.at[idx].add(src)

def _segment_sum(src, seg, n):
    return jax.ops.segment_sum(src, seg, n)

class _Rng:

    def __init__(self, key):
        self._k = key

    def _next(self):
        self._k, sub = jax.random.split(self._k)
        return sub

    def normal(self, shape):
        return jax.random.normal(self._next(), shape, dtype=jnp.bfloat16)

    def randint(self, lo, hi, shape):
        return jax.random.randint(self._next(), shape, lo, hi, dtype=jnp.int32)

    def uniform(self, shape, lo=0.0, hi=1.0):
        return jax.random.uniform(self._next(), shape, jnp.bfloat16, lo, hi)

    def permutation(self, n):
        return jax.random.permutation(self._next(), n)
kernel_name = 'sequential_preLN__memory_aug_infini_attn__moe_arch_mod__prompt'

def setup_inputs():
    _rng = _Rng(jax.random.key(int.from_bytes(__import__("os").urandom(4), "little")))
    _w = lambda a: (lambda t: t.astype(jnp.bfloat16) if jnp.issubdtype(t.dtype, jnp.floating) else t)(jnp.asarray(a))

    def _A_setup():
        B, S, D, H = (1, 2048, 576, 32)
        N = 4
        L = max(1, S // N)
        sc = D ** (-0.5)
        return {'x': _w((lambda *s: _rng.normal(s) * 0.05)(B, N * L, D)), 'wq': _w((lambda *s: _rng.normal(s) * 0.05)(D, D) * sc), 'wk': _w((lambda *s: _rng.normal(s) * 0.05)(D, D) * sc), 'wv': _w((lambda *s: _rng.normal(s) * 0.05)(D, D) * sc), 'wo': _w((lambda *s: _rng.normal(s) * 0.05)(D, D) * sc), 'beta': _w((lambda *s: _rng.normal(s) * 0.05)(H))}
    _A_in = _A_setup()

    def _B_setup():
        B, S, D, F, C = (1, 2048, 576, 4608, 1)
        return {'x': _w((lambda *s: _rng.normal(s) * 0.05)(B, S, D)), 'w_r': _w((lambda *s: _rng.normal(s) * 0.05)(D)), 'w_gate': _w((lambda *s: _rng.normal(s) * 0.05)(D, F)), 'w_up': _w((lambda *s: _rng.normal(s) * 0.05)(D, F)), 'w_down': _w((lambda *s: _rng.normal(s) * 0.05)(F, D))}
    _B_in = _B_setup()
    return {'A_x': _A_in['x'], 'A_wq': _A_in['wq'], 'A_wk': _A_in['wk'], 'A_wv': _A_in['wv'], 'A_wo': _A_in['wo'], 'A_beta': _A_in['beta'], 'B_x': _B_in['x'], 'B_w_r': _B_in['w_r'], 'B_w_gate': _B_in['w_gate'], 'B_w_up': _B_in['w_up'], 'B_w_down': _B_in['w_down']}

def reference(A_x, A_wq, A_wk, A_wv, A_wo, A_beta, B_x, B_w_r, B_w_gate, B_w_up, B_w_down):

    def _A_ref(x, wq, wk, wv, wo, beta):
        B, S, D = x.shape
        H = 32
        Dh = D // H
        N = 4
        L = S // N
        q = (lambda x, *d: x.transpose(*d))((x @ wq).reshape(B, S, H, Dh), 0, 2, 1, 3).reshape(B, H, N, L, Dh)
        k = (lambda x, *d: x.transpose(*d))((x @ wk).reshape(B, S, H, Dh), 0, 2, 1, 3).reshape(B, H, N, L, Dh)
        v = (lambda x, *d: x.transpose(*d))((x @ wv).reshape(B, S, H, Dh), 0, 2, 1, 3).reshape(B, H, N, L, Dh)
        phi = lambda t: jnp.where(t > 0, t + 1.0, jnp.exp(t))
        scale = Dh ** (-0.5)
        ar = jnp.arange(L)
        mask = (lambda x, dt: x.astype(dt))(ar[:, None] < ar[None, :], x.dtype) * -1000000000.0
        g = _sigmoid(beta).reshape(1, H, 1, 1)
        M = jnp.einsum('bhd,bhe->bhde', q[:, :, 0, 0, :] * 0.0, q[:, :, 0, 0, :] * 0.0)
        z = q[:, :, 0, 0, :] * 0.0
        outs = []
        for s in range(N):
            qs, ks, vs = (q[:, :, s].copy(), k[:, :, s].copy(), v[:, :, s].copy())
            logits = jnp.einsum('bhqd,bhkd->bhqk', qs, ks) * scale + mask
            p = _softmax(logits, axis=-1)
            a_dot = jnp.einsum('bhqk,bhkd->bhqd', p, vs)
            pq = phi(qs)
            num = jnp.einsum('bhld,bhde->bhle', pq, M)
            den = jnp.einsum('bhld,bhd->bhl', pq, z)[..., None] + 1e-06
            a_mem = num / den
            o = g * a_mem + (1.0 - g) * a_dot
            outs.append(o)
            pk = phi(ks)
            M = M + jnp.einsum('bhld,bhle->bhde', pk, vs)
            z = z + jnp.einsum('bhld->bhd', pk)
        o = (lambda x, *d: x.transpose(*d))(jnp.stack(outs, 2).reshape(B, H, S, Dh), 0, 2, 1, 3).reshape(B, S, D)
        return o @ wo

    def _B_ref(x, w_r, w_gate, w_up, w_down):
        B, S, D = x.shape
        C = 1
        r = x @ w_r
        idx = jnp.argsort(-r, axis=-1)[:, :C]
        idx_e = jnp.repeat(idx.reshape(B, C, 1), D, axis=2)
        x_sel = jnp.take_along_axis(x, idx_e, axis=1)
        g = _silu(x_sel @ w_gate)
        u = x_sel @ w_up
        y = g * u @ w_down
        r_sel = _sigmoid(jnp.take_along_axis(r, idx, axis=1))
        y = y * r_sel.reshape(B, C, 1)
        b_off = (jnp.arange(B) * S).reshape(B, 1)
        flat_idx = (idx + b_off).reshape(B * C)
        zero = (x * 0.0).reshape(B * S, D)
        upd = _scatter_add(zero, flat_idx, y.reshape(B * C, D), axis=0)
        return x + upd.reshape(B, S, D)
    x = A_x
    h = x + _A_ref(_layernorm(x, axis=-1), A_wq, A_wk, A_wv, A_wo, A_beta)
    h2 = h + _B_ref(_layernorm(h, axis=-1), B_w_r, B_w_gate, B_w_up, B_w_down)
    return h2
```

```python
import math

import jax
import jax.numpy as jnp
from jax import lax
import jax.experimental.pallas as pl
import jax.experimental.pallas.tpu as pltpu

bf16 = jnp.bfloat16
f32 = jnp.float32
u32 = jnp.uint32

S, D, H, DH, NSEG, L, F = 2048, 576, 32, 18, 4, 512, 4608
G = 5
GW = 126
GR = (128, 128, 128, 128, 80)
GO = (0, 128, 256, 384, 512)
NP = 592
NT = L // 128
OFF = (0, 128, 384, 768)
EPS = 1e-5
QSCALE = (DH ** -0.5) * math.log2(math.e)
ONE_LO = 0x00003F80
FCH = 512

_NT = (((1,), (1,)), ((), ()))


def _phi(t):
    return jnp.where(t > 0, t + 1.0, jnp.exp(t))


def _ln0(v):
    m = jnp.mean(v, axis=0, keepdims=True)
    c = v - m
    var = jnp.mean(c * c, axis=0, keepdims=True)
    return c * lax.rsqrt(var + EPS)


def _kernel(x_hbm, wq_hbm, wk_hbm, wv_hbm, wo_hbm, beta_ref, wr_ref, wg_hbm, wu_hbm, wd_hbm,
            out_hbm,
            xbuf, wq_v, wk_v, wv_v, wo_v, wg_v, wu_v, wd_v,
            wall, wo_t, wr_tab,
            k_buf, pk_buf, q_buf, pq_buf, v_buf,
            s0, s1, m0, m1, am_buf, o_buf, gm_tab, g_tab,
            m_st, h_buf, obuf,
            sems):
    def x_copy(s):
        return pltpu.make_async_copy(x_hbm.at[0, :, pl.ds(s * L, L)], xbuf.at[s], sems.at[s])
    cp_wk = pltpu.make_async_copy(wk_hbm, wk_v, sems.at[4])
    cp_wq = pltpu.make_async_copy(wq_hbm, wq_v, sems.at[5])
    cp_wv = pltpu.make_async_copy(wv_hbm, wv_v, sems.at[6])
    cp_wo = pltpu.make_async_copy(wo_hbm, wo_v, sems.at[7])
    cp_wg = pltpu.make_async_copy(wg_hbm, wg_v, sems.at[8])
    cp_wu = pltpu.make_async_copy(wu_hbm, wu_v, sems.at[9])
    cp_wd = pltpu.make_async_copy(wd_hbm, wd_v, sems.at[10])

    def o_copy(s):
        return pltpu.make_async_copy(obuf.at[s], out_hbm.at[0, :, pl.ds(s * L, L)], sems.at[11 + s])

    cp_wq.start(); cp_wk.start(); cp_wv.start(); x_copy(0).start(); cp_wo.start()
    for s in range(1, NSEG):
        x_copy(s).start()
    cp_wg.start(); cp_wu.start(); cp_wd.start()

    gate = jax.nn.sigmoid(beta_ref[...].astype(f32).reshape(1, H))
    rowi = lax.broadcasted_iota(jnp.int32, (640, H), 0)
    coli = lax.broadcasted_iota(jnp.int32, (640, H), 1)
    gcol = jnp.sum(jnp.where((rowi >= coli * DH) & (rowi < coli * DH + DH), gate, 0.0), axis=1, keepdims=True)
    gfull = jnp.broadcast_to(gcol, (640, 128))
    gm_tab[...] = 1.0 - gfull
    g_tab[...] = gfull
    wr_tab[...] = jnp.broadcast_to(wr_ref[...].astype(f32).reshape(1, D), (128, D)).T
    am_buf[...] = jnp.zeros_like(am_buf)
    m_st[...] = jnp.zeros_like(m_st)
    o_buf[...] = jnp.zeros_like(o_buf)
    v_buf[...] = jnp.zeros_like(v_buf)
    pq_buf[...] = jnp.zeros_like(pq_buf)
    pk_buf[...] = jnp.zeros_like(pk_buf)
    k_buf[...] = jnp.zeros_like(k_buf)

    def put_padded(w_ref, base):
        wT = w_ref[...].astype(f32).T
        for g in range(G):
            w = min(GW, D - g * GW)
            blk = jnp.concatenate([wT[g * GW:g * GW + w], jnp.zeros((GR[g] - w, D), f32)], axis=0)
            wall[base + GO[g]:base + GO[g] + GR[g], :] = blk.astype(bf16)
    cp_wq.wait()
    put_padded(wq_v, 0)
    cp_wk.wait()
    put_padded(wk_v, NP)
    cp_wv.wait()
    wall[2 * NP:2 * NP + D, :] = wv_v[...].astype(f32).T.astype(bf16)
    cp_wo.wait()
    wo_t[...] = wo_v[...].astype(f32).T.astype(bf16)

    row64 = lax.broadcasted_iota(jnp.int32, (64, 128), 0)
    vrow = lax.broadcasted_iota(jnp.int32, (16, 128), 0)
    kk = lax.broadcasted_iota(jnp.int32, (128, 128), 0)
    qq = lax.broadcasted_iota(jnp.int32, (128, 128), 1)
    causal = kk <= qq
    bd = jnp.zeros((128, 128), jnp.bool_)
    for r in range(7):
        bd = bd | ((kk >= r * DH) & (kk < r * DH + DH) & (qq >= r * DH) & (qq < r * DH + DH))
    lane = lax.broadcasted_iota(jnp.int32, (1, 128), 1)

    def qk(h, s_buf, m_buf):
        g = h // 7
        r = h - g * 7
        qmask = (row64 >= 9 * r) & (row64 < 9 * r + 9)
        for j in range(NT):
            n = 128 * (j + 1)
            qt = pltpu.bitcast(jnp.where(qmask, q_buf[g, j], jnp.uint32(0)), bf16)
            kt = pltpu.bitcast(k_buf[g, 0:n // 2, :], bf16)
            s = jnp.dot(kt, qt, preferred_element_type=f32)
            sd = jnp.where(causal, s[n - 128:], -1e30)
            mx = jnp.max(sd.reshape(16, 8, 128), axis=0)
            s_buf[OFF[j] + n - 128:OFF[j] + n, :] = sd
            if j > 0:
                s_buf[OFF[j]:OFF[j] + n - 128, :] = s[:n - 128]
                mx = jnp.maximum(mx, jnp.max(s[:n - 128].reshape(16 * j, 8, 128), axis=0))
            m_buf[j] = mx

    def pv(h, s_buf, m_buf):
        gm = gm_tab[pl.ds(DH * h, 24), :]
        for j in range(NT):
            n = 128 * (j + 1)
            m = jnp.max(m_buf[j], axis=0, keepdims=True)
            p = jnp.exp2(s_buf[OFF[j]:OFF[j] + n, :] - m).astype(bf16)
            vs = []
            for kb in range(j + 1):
                vv = v_buf[kb, pl.ds(9 * h, 16), :]
                vv = jnp.where(vrow == 9, jnp.uint32(ONE_LO), vv)
                vs.append(pltpu.bitcast(vv, bf16))
            va = jnp.concatenate(vs, axis=1) if j > 0 else vs[0]
            o = jnp.dot(va, p, preferred_element_type=f32)
            o = o[:24] * (gm / o[18:19]) + am_buf[j, pl.ds(DH * h, 24), :]
            o_buf[j, pl.ds(DH * h, 24), :] = o

    def segment(s, carry):
        x_copy(s).wait()
        for j in range(NT):
            xn = _ln0(xbuf[s, :, j * 128:(j + 1) * 128].astype(f32)).astype(bf16)
            t = jnp.dot(wall[...], xn, preferred_element_type=f32)
            for g in range(G):
                qg = t[GO[g]:GO[g] + GR[g]]
                q_buf[g, j, 0:GR[g] // 2, :] = pltpu.bitcast((qg * QSCALE).astype(bf16), u32)
                pq_buf[g, j, 0:GR[g] // 2, :] = pltpu.bitcast(_phi(qg).astype(bf16), u32)
                kg = t[NP + GO[g]:NP + GO[g] + GR[g]]
                pk_buf[g, j, 0:GR[g] // 2, :] = pltpu.bitcast(_phi(kg).astype(bf16), u32)
                if GR[g] < 128:
                    kg = jnp.concatenate([kg, jnp.zeros((128 - GR[g], 128), f32)], axis=0)
                k_buf[g, 64 * j:64 * (j + 1), :] = pltpu.bitcast(kg.T.astype(bf16), u32)
            v_buf[j, 0:D // 2, :] = pltpu.bitcast(t[2 * NP:].astype(bf16), u32)

        @pl.when(s > 0)
        def _():
            for g in range(G):
                mb = jnp.where(bd, m_st[g, 0:128, :], 0.0).astype(bf16)
                zb = jnp.where(bd, m_st[g, 128:129, :], 0.0).astype(bf16)
                lhs = jnp.concatenate([mb, zb], axis=0)
                gg = g_tab[pl.ds(g * GW, 128), :]
                for j in range(NT):
                    rr = jnp.dot(lhs, pltpu.bitcast(pq_buf[g, j], bf16), preferred_element_type=f32)
                    am_buf[j, g * GW:g * GW + 128, :] = gg * (rr[:128] / (rr[128:] + 1e-6))

        qk(0, s0, m0)

        def head(i, c):
            qk(2 * i + 1, s1, m1)
            pv(2 * i, s0, m0)
            qk(2 * i + 2, s0, m0)
            pv(2 * i + 1, s1, m1)
            return c
        lax.fori_loop(0, H // 2 - 1, head, 0)
        qk(H - 1, s1, m1)
        pv(H - 2, s0, m0)
        pv(H - 1, s1, m1)

        @pl.when(s < NSEG - 1)
        def _():
            ones = jnp.ones((16, 128), bf16)
            for g in range(G):
                acc = m_st[g]
                for kb in range(NT):
                    vg = jnp.concatenate([pltpu.bitcast(v_buf[kb, g * 63:g * 63 + 64, :], bf16), ones], axis=0)
                    acc = acc + lax.dot_general(vg, pltpu.bitcast(pk_buf[g, kb], bf16), _NT,
                                                preferred_element_type=f32)
                m_st[g] = acc

        rbest, ibest = carry
        for j in range(NT):
            att = jnp.dot(wo_t[...], o_buf[j, 0:D, :].astype(bf16), preferred_element_type=f32)
            hh = xbuf[s, :, j * 128:(j + 1) * 128].astype(f32) + att
            ln = _ln0(hh)
            obuf[s, :, j * 128:(j + 1) * 128] = (hh + ln).astype(bf16)
            h_buf[s * NT + j] = hh
            r = jnp.sum(ln * wr_tab[...], axis=0, keepdims=True)
            take = r > rbest
            rbest = jnp.where(take, r, rbest)
            ibest = jnp.where(take, lane + (s * L + j * 128), ibest)
        o_copy(s).start()
        return rbest, ibest

    rbest, ibest = lax.fori_loop(
        0, NSEG, segment, (jnp.full((1, 128), -jnp.inf, f32), jnp.zeros((1, 128), jnp.int32)))

    rmax = jnp.max(rbest, axis=1, keepdims=True)
    imin = jnp.min(jnp.where(rbest == rmax, ibest, S), axis=1, keepdims=True)
    idx = imin[0, 0]
    tile = idx // 128
    onehot = _NB = (lane == imin - (imin // 128) * 128)
    hh = h_buf[tile]
    ln = _ln0(hh)
    oh = jnp.broadcast_to(jnp.where(onehot, 1.0, 0.0), (16, 128)).astype(bf16)
    xs = lax.dot_general(oh, ln.astype(bf16), _NT, preferred_element_type=f32).astype(bf16)
    cp_wg.wait(); cp_wu.wait(); cp_wd.wait()
    y = jnp.zeros((D, 128), f32)
    for c in range(F // FCH):
        cs = slice(c * FCH, (c + 1) * FCH)
        gt = jnp.dot(xs, wg_v[:, cs], preferred_element_type=f32)
        up = jnp.dot(xs, wu_v[:, cs], preferred_element_type=f32)
        act = (gt * jax.nn.sigmoid(gt) * up).astype(bf16).astype(f32)[0:1]
        pr = wd_v[:, cs].astype(f32) * act
        for cc in range(FCH // 128):
            y = y + pr[:, cc * 128:(cc + 1) * 128]
    y = jnp.sum(y, axis=1, keepdims=True) * jax.nn.sigmoid(rmax)
    new_tile = jnp.where(onehot, hh + (ln + y), hh + ln).astype(bf16)
    for s in range(NSEG):
        o_copy(s).wait()
    obuf[0, :, 0:128] = new_tile
    fin = pltpu.make_async_copy(obuf.at[0, :, 0:128],
                                out_hbm.at[0, :, pl.ds(pl.multiple_of(tile * 128, 128), 128)], sems.at[15])
    fin.start()
    fin.wait()


@jax.jit
def pallas_sequential_preLN__memory_aug_infini_attn__moe_arch_mod__prompt_kernel(
    A_x: jax.Array,
    A_wq: jax.Array,
    A_wk: jax.Array,
    A_wv: jax.Array,
    A_wo: jax.Array,
    A_beta: jax.Array,
    B_x: jax.Array,
    B_w_r: jax.Array,
    B_w_gate: jax.Array,
    B_w_up: jax.Array,
    B_w_down: jax.Array,
):
    hbm = pl.BlockSpec(memory_space=pltpu.HBM)
    vmem_spec = pl.BlockSpec(memory_space=pltpu.VMEM)
    V = pltpu.VMEM
    scratch = [
        V((NSEG, D, L), bf16),
        V((D, D), bf16), V((D, D), bf16), V((D, D), bf16), V((D, D), bf16),
        V((D, F), bf16), V((D, F), bf16), V((D, F), bf16),
        V((2 * NP + D, D), bf16), V((D, D), bf16), V((D, 128), f32),
        V((G, L // 2, 128), u32), V((G, NT, 64, 128), u32),
        V((G, NT, 64, 128), u32), V((G, NT, 64, 128), u32),
        V((NT, 320, 128), u32),
        V((1280, 128), f32), V((1280, 128), f32), V((NT, 8, 128), f32), V((NT, 8, 128), f32),
        V((NT, 640, 128), f32), V((NT, 640, 128), f32), V((640, 128), f32), V((640, 128), f32),
        V((G, 144, 128), f32),
        V((S // 128, D, 128), f32), V((NSEG, D, L), bf16),
        pltpu.SemaphoreType.DMA((16,)),
    ]
    out_t = pl.pallas_call(
        _kernel,
        out_shape=jax.ShapeDtypeStruct((1, D, S), A_x.dtype),
        in_specs=[hbm] * 5 + [vmem_spec, vmem_spec] + [hbm] * 3,
        out_specs=hbm,
        scratch_shapes=scratch,
        compiler_params=pltpu.CompilerParams(vmem_limit_bytes=100 * 1024 * 1024),
    )(jnp.swapaxes(A_x, 1, 2), A_wq, A_wk, A_wv, A_wo, A_beta, B_w_r, B_w_gate, B_w_up, B_w_down.T)
    return jnp.swapaxes(out_t, 1, 2)
```

```python
import math

import jax
import jax.numpy as jnp
from jax import lax
import jax.experimental.pallas as pl
import jax.experimental.pallas.tpu as pltpu

bf16 = jnp.bfloat16
f32 = jnp.float32
u32 = jnp.uint32

S, D, H, DH, NSEG, L, F = 2048, 576, 32, 18, 4, 512, 4608
G = 5
GW = 126
GR = (128, 128, 128, 128, 80)
GO = (0, 128, 256, 384, 512)
NP = 592
NT = L // 128
OFF = (0, 128, 384, 768)
EPS = 1e-5
QSCALE = (DH ** -0.5) * math.log2(math.e)
ONE_LO = 0x00003F80
FCH = 512
HU = 10

_NT = (((1,), (1,)), ((), ()))


def _phi(t):
    return jnp.where(t > 0, t + 1.0, jnp.exp(t))


def _ln0(v):
    m = jnp.mean(v, axis=0, keepdims=True)
    c = v - m
    var = jnp.mean(c * c, axis=0, keepdims=True)
    return c * lax.rsqrt(var + EPS)


def _kernel(x_hbm, wq_hbm, wk_hbm, wv_hbm, wo_hbm, beta_ref, wr_ref, wg_hbm, wu_hbm, wd_hbm,
            out_hbm,
            xbuf, wq_v, wk_v, wv_v, wo_v, wg_v, wu_v, wd_v,
            wall, wo_t, wr_tab,
            k_buf, pk_buf, q_buf, pq_buf, v_buf,
            s0, s1, m0, m1, am_buf, o_buf, gm_tab, g_tab,
            m_st, h_buf, obuf,
            sems):
    def x_copy(s):
        return pltpu.make_async_copy(x_hbm.at[0, :, pl.ds(s * L, L)], xbuf.at[s], sems.at[s])
    cp_wk = pltpu.make_async_copy(wk_hbm, wk_v, sems.at[4])
    cp_wq = pltpu.make_async_copy(wq_hbm, wq_v, sems.at[5])
    cp_wv = pltpu.make_async_copy(wv_hbm, wv_v, sems.at[6])
    cp_wo = pltpu.make_async_copy(wo_hbm, wo_v, sems.at[7])
    cp_wg = pltpu.make_async_copy(wg_hbm, wg_v, sems.at[8])
    cp_wu = pltpu.make_async_copy(wu_hbm, wu_v, sems.at[9])
    cp_wd = pltpu.make_async_copy(wd_hbm, wd_v, sems.at[10])

    def o_copy(s):
        return pltpu.make_async_copy(obuf.at[s], out_hbm.at[0, :, pl.ds(s * L, L)], sems.at[11 + s])

    x_copy(0).start(); cp_wq.start(); cp_wk.start(); cp_wv.start(); cp_wo.start()
    for s in range(1, NSEG):
        x_copy(s).start()
    cp_wg.start(); cp_wu.start(); cp_wd.start()

    gate = jax.nn.sigmoid(beta_ref[...].astype(f32).reshape(1, H))
    rowi = lax.broadcasted_iota(jnp.int32, (640, H), 0)
    coli = lax.broadcasted_iota(jnp.int32, (640, H), 1)
    gcol = jnp.sum(jnp.where((rowi >= coli * DH) & (rowi < coli * DH + DH), gate, 0.0), axis=1, keepdims=True)
    gfull = jnp.broadcast_to(gcol, (640, 128))
    gm_tab[...] = 1.0 - gfull
    g_tab[...] = gfull
    wr_tab[...] = jnp.broadcast_to(wr_ref[...].astype(f32).reshape(1, D), (128, D)).T
    am_buf[...] = jnp.zeros_like(am_buf)
    m_st[...] = jnp.zeros_like(m_st)
    o_buf[...] = jnp.zeros_like(o_buf)
    v_buf[...] = jnp.zeros_like(v_buf)
    pq_buf[...] = jnp.zeros_like(pq_buf)
    pk_buf[...] = jnp.zeros_like(pk_buf)
    k_buf[...] = jnp.zeros_like(k_buf)

    def put_padded(w_ref, base):
        wT = pltpu.bitcast(w_ref[...].T, u32)
        for g in range(G):
            w = min(GW, D - g * GW) // 2
            r0 = (base + GO[g]) // 2
            wall[r0:r0 + w, :] = wT[g * 63:g * 63 + w]
            wall[r0 + w:r0 + GR[g] // 2, :] = jnp.zeros((GR[g] // 2 - w, D), u32)

    row64 = lax.broadcasted_iota(jnp.int32, (64, 128), 0)
    vrow = lax.broadcasted_iota(jnp.int32, (16, 128), 0)
    kk = lax.broadcasted_iota(jnp.int32, (128, 128), 0)
    qq = lax.broadcasted_iota(jnp.int32, (128, 128), 1)
    causal = kk <= qq
    bd = jnp.zeros((128, 128), jnp.bool_)
    for r in range(7):
        bd = bd | ((kk >= r * DH) & (kk < r * DH + DH) & (qq >= r * DH) & (qq < r * DH + DH))
    lane = lax.broadcasted_iota(jnp.int32, (1, 128), 1)
    zr = lax.broadcasted_iota(jnp.int32, (16, 128), 0)
    zc = lax.broadcasted_iota(jnp.int32, (16, 128), 1)
    zmask = (zc >= zr * DH) & (zc < zr * DH + DH)

    def qk(h, s_buf, m_buf):
        g = h // 7
        r = h - g * 7
        qmask = (row64 >= 9 * r) & (row64 < 9 * r + 9)
        for j in range(NT):
            n = 128 * (j + 1)
            qt = pltpu.bitcast(jnp.where(qmask, q_buf[g, j], jnp.uint32(0)), bf16)
            kt = pltpu.bitcast(k_buf[g, 0:n // 2, :], bf16)
            s = jnp.dot(kt, qt, preferred_element_type=f32)
            sd = jnp.where(causal, s[n - 128:], -1e30)
            mx = jnp.max(sd.reshape(16, 8, 128), axis=0)
            s_buf[OFF[j] + n - 128:OFF[j] + n, :] = sd
            if j > 0:
                s_buf[OFF[j]:OFF[j] + n - 128, :] = s[:n - 128]
                mx = jnp.maximum(mx, jnp.max(s[:n - 128].reshape(16 * j, 8, 128), axis=0))
            m_buf[j] = mx

    def pv(h, s_buf, m_buf):
        gm = gm_tab[pl.ds(DH * h, 24), :]
        for j in range(NT):
            n = 128 * (j + 1)
            m = jnp.max(m_buf[j], axis=0, keepdims=True)
            p = jnp.exp2(s_buf[OFF[j]:OFF[j] + n, :] - m).astype(bf16)
            vs = []
            for kb in range(j + 1):
                vv = v_buf[kb, pl.ds(9 * h, 16), :]
                vv = jnp.where(vrow == 9, jnp.uint32(ONE_LO), vv)
                vs.append(pltpu.bitcast(vv, bf16))
            va = jnp.concatenate(vs, axis=1) if j > 0 else vs[0]
            o = jnp.dot(va, p, preferred_element_type=f32)
            o = (o[:24] * gm) * (1.0 / o[18:19]) + am_buf[j, pl.ds(DH * h, 24), :]
            o_buf[j, pl.ds(DH * h, 24), :] = o

    def ln_in(s, j):
        return _ln0(xbuf[s, :, j * 128:(j + 1) * 128].astype(f32)).astype(bf16)

    def proj_q(xn, j):
        t = jnp.dot(pltpu.bitcast(wall[0:NP // 2, :], bf16), xn, preferred_element_type=f32)
        for g in range(G):
            qg = t[GO[g]:GO[g] + GR[g]]
            q_buf[g, j, 0:GR[g] // 2, :] = pltpu.bitcast((qg * QSCALE).astype(bf16), u32)
            pq_buf[g, j, 0:GR[g] // 2, :] = pltpu.bitcast(_phi(qg).astype(bf16), u32)

    def proj_k(xn, j):
        t = jnp.dot(pltpu.bitcast(wall[NP // 2:NP, :], bf16), xn, preferred_element_type=f32)
        for g in range(G):
            kg = t[GO[g]:GO[g] + GR[g]]
            pk_buf[g, j, 0:GR[g] // 2, :] = pltpu.bitcast(_phi(kg).astype(bf16), u32)
            kb = kg.astype(bf16)
            if GR[g] < 128:
                kb = jnp.concatenate([kb, jnp.zeros((128 - GR[g], 128), bf16)], axis=0)
            k_buf[g, 64 * j:64 * (j + 1), :] = pltpu.bitcast(kb.T, u32)

    def proj_v(xn, j):
        t = jnp.dot(pltpu.bitcast(wall[NP:NP + D // 2, :], bf16), xn, preferred_element_type=f32)
        v_buf[j, 0:D // 2, :] = pltpu.bitcast(t.astype(bf16), u32)

    def retrieve():
        r8 = lax.broadcasted_iota(jnp.int32, (8, 128), 0)
        for g in range(G):
            mb = jnp.where(bd, m_st[g, 0:128, :], 0.0).astype(bf16)
            zb = jnp.where(zmask, m_st[g, 128:129, :], 0.0).astype(bf16)
            lhs = jnp.concatenate([mb[:GR[g]], zb], axis=0)
            for j in range(NT):
                rr = jnp.dot(lhs, pltpu.bitcast(pq_buf[g, j], bf16), preferred_element_type=f32)
                rd = 1.0 / (rr[GR[g]:GR[g] + 8] + 1e-6)
                rb = [jnp.broadcast_to(rd[i:i + 1], (8, 128)) for i in range(8)]
                for v in range(GR[g] // 8):
                    h1, h2 = (8 * v) // DH, (8 * v + 7) // DH
                    e = rb[h1] if h1 == h2 else jnp.where(r8 < h2 * DH - 8 * v, rb[h1], rb[h2])
                    gg = g_tab[g * GW + 8 * v:g * GW + 8 * v + 8, :]
                    am_buf[j, g * GW + 8 * v:g * GW + 8 * v + 8, :] = (gg * rr[8 * v:8 * v + 8]) * e

    def update():
        ones = jnp.ones((16, 128), bf16)
        for g in range(G):
            n = GR[g]
            acc = m_st[g]
            for kb in range(NT):
                vg = jnp.concatenate([pltpu.bitcast(v_buf[kb, g * 63:g * 63 + 64, :], bf16), ones], axis=0)
                acc = acc + lax.dot_general(vg, pltpu.bitcast(pk_buf[g, kb], bf16), _NT,
                                            preferred_element_type=f32)
            m_st[g] = acc

    def out_tile(s, j, rbest, ibest):
        att = jnp.dot(pltpu.bitcast(wo_t[...], bf16), o_buf[j, 0:D, :].astype(bf16), preferred_element_type=f32)
        hh = xbuf[s, :, j * 128:(j + 1) * 128].astype(f32) + att
        ln = _ln0(hh)
        obuf[s, :, j * 128:(j + 1) * 128] = (hh + ln).astype(bf16)
        h_buf[s * NT + j] = hh
        r = jnp.sum(ln * wr_tab[...], axis=0, keepdims=True)
        take = r > rbest
        return jnp.where(take, r, rbest), jnp.where(take, lane + (s * L + j * 128), ibest)

    x_copy(0).wait()
    xns = [ln_in(0, j) for j in range(NT)]
    cp_wq.wait()
    put_padded(wq_v, 0)
    for j in range(NT):
        proj_q(xns[j], j)
    cp_wk.wait()
    put_padded(wk_v, NP)
    for j in range(NT):
        proj_k(xns[j], j)
    cp_wv.wait()
    wall[NP:NP + D // 2, :] = pltpu.bitcast(wv_v[...].T, u32)
    for j in range(NT):
        proj_v(xns[j], j)
    cp_wo.wait()
    wo_t[...] = pltpu.bitcast(wo_v[...].T, u32)
    qk(0, s0, m0)

    def segment(s, carry):
        def heads(i, c):
            for a in range(HU // 2):
                h = i * HU + 2 * a
                qk(h + 1, s1, m1)
                pv(h, s0, m0)
                qk(h + 2, s0, m0)
                pv(h + 1, s1, m1)
            return c
        lax.fori_loop(0, (H - 2) // HU, heads, 0)

        def finish(rbest, ibest):
            qk(H - 1, s1, m1)
            pv(H - 2, s0, m0)
            pv(H - 1, s1, m1)
            return rbest, ibest

        def mid(rbest, ibest):
            finish(rbest, ibest)
            update()
            x_copy(s + 1).wait()
            for j in range(NT):
                rbest, ibest = out_tile(s, j, rbest, ibest)
            o_copy(s).start()
            for j in range(NT):
                xn = ln_in(s + 1, j)
                proj_q(xn, j)
                proj_k(xn, j)
                proj_v(xn, j)
            retrieve()
            qk(0, s0, m0)
            return rbest, ibest

        def last(rbest, ibest):
            finish(rbest, ibest)
            for j in range(NT):
                rbest, ibest = out_tile(s, j, rbest, ibest)
            o_copy(s).start()
            return rbest, ibest

        return lax.cond(s < NSEG - 1, mid, last, *carry)

    rbest, ibest = lax.fori_loop(
        0, NSEG, segment, (jnp.full((1, 128), -jnp.inf, f32), jnp.zeros((1, 128), jnp.int32)))

    rmax = jnp.max(rbest, axis=1, keepdims=True)
    imin = jnp.min(jnp.where(rbest == rmax, ibest, S), axis=1, keepdims=True)
    idx = imin[0, 0]
    tile = idx // 128
    onehot = _NB = (lane == imin - (imin // 128) * 128)
    hh = h_buf[tile]
    ln = _ln0(hh)
    oh = jnp.broadcast_to(jnp.where(onehot, 1.0, 0.0), (16, 128)).astype(bf16)
    xs = lax.dot_general(oh, ln.astype(bf16), _NT, preferred_element_type=f32).astype(bf16)
    cp_wg.wait(); cp_wu.wait(); cp_wd.wait()
    y = jnp.zeros((D, 128), f32)
    for c in range(F // FCH):
        cs = slice(c * FCH, (c + 1) * FCH)
        gt = jnp.dot(xs, wg_v[:, cs], preferred_element_type=f32)
        up = jnp.dot(xs, wu_v[:, cs], preferred_element_type=f32)
        act = (gt * jax.nn.sigmoid(gt) * up).astype(bf16).astype(f32)[0:1]
        pr = wd_v[:, cs].astype(f32) * act
        for cc in range(FCH // 128):
            y = y + pr[:, cc * 128:(cc + 1) * 128]
    y = jnp.sum(y, axis=1, keepdims=True) * jax.nn.sigmoid(rmax)
    new_tile = jnp.where(onehot, hh + (ln + y), hh + ln).astype(bf16)
    for s in range(NSEG):
        o_copy(s).wait()
    obuf[0, :, 0:128] = new_tile
    fin = pltpu.make_async_copy(obuf.at[0, :, 0:128],
                                out_hbm.at[0, :, pl.ds(pl.multiple_of(tile * 128, 128), 128)], sems.at[15])
    fin.start()
    fin.wait()


@jax.jit
def pallas_sequential_preLN__memory_aug_infini_attn__moe_arch_mod__prompt_kernel(
    A_x: jax.Array,
    A_wq: jax.Array,
    A_wk: jax.Array,
    A_wv: jax.Array,
    A_wo: jax.Array,
    A_beta: jax.Array,
    B_x: jax.Array,
    B_w_r: jax.Array,
    B_w_gate: jax.Array,
    B_w_up: jax.Array,
    B_w_down: jax.Array,
):
    hbm = pl.BlockSpec(memory_space=pltpu.HBM)
    vmem_spec = pl.BlockSpec(memory_space=pltpu.VMEM)
    V = pltpu.VMEM
    scratch = [
        V((NSEG, D, L), bf16),
        V((D, D), bf16), V((D, D), bf16), V((D, D), bf16), V((D, D), bf16),
        V((D, F), bf16), V((D, F), bf16), V((D, F), bf16),
        V((NP + D // 2, D), u32), V((D // 2, D), u32), V((D, 128), f32),
        V((G, L // 2, 128), u32), V((G, NT, 64, 128), u32),
        V((G, NT, 64, 128), u32), V((G, NT, 64, 128), u32),
        V((NT, 320, 128), u32),
        V((1280, 128), f32), V((1280, 128), f32), V((NT, 8, 128), f32), V((NT, 8, 128), f32),
        V((NT, 640, 128), f32), V((NT, 640, 128), f32), V((640, 128), f32), V((640, 128), f32),
        V((G, 144, 128), f32),
        V((S // 128, D, 128), f32), V((NSEG, D, L), bf16),
        pltpu.SemaphoreType.DMA((16,)),
    ]
    out_t = pl.pallas_call(
        _kernel,
        out_shape=jax.ShapeDtypeStruct((1, D, S), A_x.dtype),
        in_specs=[hbm] * 5 + [vmem_spec, vmem_spec] + [hbm] * 3,
        out_specs=hbm,
        scratch_shapes=scratch,
        compiler_params=pltpu.CompilerParams(vmem_limit_bytes=100 * 1024 * 1024),
    )(jnp.swapaxes(A_x, 1, 2), A_wq, A_wk, A_wv, A_wo, A_beta, B_w_r, B_w_gate, B_w_up, B_w_down.T)
    return jnp.swapaxes(out_t, 1, 2)
```

```python
import math

import jax
import jax.numpy as jnp
from jax import lax
import jax.experimental.pallas as pl
import jax.experimental.pallas.tpu as pltpu

bf16 = jnp.bfloat16
f32 = jnp.float32
u32 = jnp.uint32

S, D, H, DH, NSEG, L, F = 2048, 576, 32, 18, 4, 512, 4608
G = 5
GW = 126
GR = (128, 128, 128, 128, 80)
GO = (0, 128, 256, 384, 512)
NP = 592
NT = L // 128
OFF = (0, 128, 384, 768)
EPS = 1e-5
QSCALE = (DH ** -0.5) * math.log2(math.e)
ONE_LO = 0x00003F80
FCH = 512
HU = 10

_NT = (((1,), (1,)), ((), ()))


def _phi(t):
    return jnp.where(t > 0, t + 1.0, jnp.exp(t))


def _sum0(v):
    t = jnp.sum(v.reshape(8, D // 8, 128), axis=0)
    t = jnp.sum(t.reshape(3, D // 24, 128), axis=0)
    t = jnp.sum(t.reshape(3, 8, 128), axis=0)
    return jnp.sum(t, axis=0, keepdims=True)


CH = 48


def _fold(acc, c):
    t = jnp.sum(c.reshape(CH // 8, 8, 128), axis=0)
    return t if acc is None else acc + t


def _stats(chunks):
    s1 = s2 = shift = None
    for c in chunks:
        if shift is None:
            shift = c[0:1]
        d = c - shift
        s1 = _fold(s1, d)
        s2 = _fold(s2, d * d)
    m1 = jnp.sum(s1, axis=0, keepdims=True) * (1.0 / D)
    m2 = jnp.sum(s2, axis=0, keepdims=True) * (1.0 / D)
    var = jnp.maximum(m2 - m1 * m1, 0.0)
    return shift + m1, lax.rsqrt(var + EPS)


def _ln0(v):
    m = _sum0(v) * (1.0 / D)
    c = v - m
    var = _sum0(c * c) * (1.0 / D)
    return c * lax.rsqrt(var + EPS)


def _kernel(x_hbm, wq_hbm, wk_hbm, wv_hbm, wo_hbm, beta_ref, wr_ref, wg_hbm, wu_hbm, wd_hbm,
            out_hbm,
            xbuf, wq_v, wk_v, wv_v, wo_v, wg_v, wu_v, wd_v,
            wall, wo_t, wr_tab,
            k_buf, pk_buf, q_buf, pq_buf, v_buf,
            s0, s1, m0, m1, am_buf, o_buf, gm_tab, g_tab,
            m_st, h_buf, l_buf, obuf,
            sems):
    def x_copy(s):
        return pltpu.make_async_copy(x_hbm.at[0, :, pl.ds(s * L, L)], xbuf.at[s], sems.at[s])
    cp_wk = pltpu.make_async_copy(wk_hbm, wk_v, sems.at[4])
    cp_wq = pltpu.make_async_copy(wq_hbm, wq_v, sems.at[5])
    cp_wv = pltpu.make_async_copy(wv_hbm, wv_v, sems.at[6])
    cp_wo = pltpu.make_async_copy(wo_hbm, wo_v, sems.at[7])
    cp_wg = pltpu.make_async_copy(wg_hbm, wg_v, sems.at[8])
    cp_wu = pltpu.make_async_copy(wu_hbm, wu_v, sems.at[9])
    cp_wd = pltpu.make_async_copy(wd_hbm, wd_v, sems.at[10])

    def o_copy(s):
        return pltpu.make_async_copy(obuf.at[s], out_hbm.at[0, :, pl.ds(s * L, L)], sems.at[11 + s])

    x_copy(0).start(); cp_wq.start(); cp_wk.start(); cp_wv.start()

    gate = jax.nn.sigmoid(beta_ref[...].astype(f32).reshape(1, H))
    rowi = lax.broadcasted_iota(jnp.int32, (640, H), 0)
    coli = lax.broadcasted_iota(jnp.int32, (640, H), 1)
    gcol = jnp.sum(jnp.where((rowi >= coli * DH) & (rowi < coli * DH + DH), gate, 0.0), axis=1, keepdims=True)
    gfull = jnp.broadcast_to(gcol, (640, 128))
    gm_tab[...] = 1.0 - gfull
    g_tab[...] = gfull
    wr_tab[...] = jnp.broadcast_to(wr_ref[...].astype(f32).reshape(1, D), (128, D)).T
    am_buf[...] = jnp.zeros_like(am_buf)
    m_st[...] = jnp.zeros_like(m_st)
    o_buf[...] = jnp.zeros_like(o_buf)
    v_buf[...] = jnp.zeros_like(v_buf)
    pq_buf[...] = jnp.zeros_like(pq_buf)
    pk_buf[...] = jnp.zeros_like(pk_buf)
    k_buf[...] = jnp.zeros_like(k_buf)

    def put_padded(w_ref, base):
        wT = pltpu.bitcast(w_ref[...].T, u32)
        for g in range(G):
            w = min(GW, D - g * GW) // 2
            r0 = (base + GO[g]) // 2
            wall[r0:r0 + w, :] = wT[g * 63:g * 63 + w]
            wall[r0 + w:r0 + GR[g] // 2, :] = jnp.zeros((GR[g] // 2 - w, D), u32)

    row64 = lax.broadcasted_iota(jnp.int32, (64, 128), 0)
    vrow = lax.broadcasted_iota(jnp.int32, (16, 128), 0)
    kk = lax.broadcasted_iota(jnp.int32, (128, 128), 0)
    qq = lax.broadcasted_iota(jnp.int32, (128, 128), 1)
    causal = kk <= qq
    bd = jnp.zeros((128, 128), jnp.bool_)
    for r in range(7):
        bd = bd | ((kk >= r * DH) & (kk < r * DH + DH) & (qq >= r * DH) & (qq < r * DH + DH))
    lane = lax.broadcasted_iota(jnp.int32, (1, 128), 1)
    zr = lax.broadcasted_iota(jnp.int32, (16, 128), 0)
    zc = lax.broadcasted_iota(jnp.int32, (16, 128), 1)
    zmask = (zc >= zr * DH) & (zc < zr * DH + DH)

    def qk(h, s_buf, m_buf):
        g = h // 7
        r = h - g * 7
        qmask = (row64 >= 9 * r) & (row64 < 9 * r + 9)
        for j in range(NT):
            n = 128 * (j + 1)
            qt = pltpu.bitcast(jnp.where(qmask, q_buf[g, j], jnp.uint32(0)), bf16)
            kt = pltpu.bitcast(k_buf[g, 0:n // 2, :], bf16)
            s = jnp.dot(kt, qt, preferred_element_type=f32)
            sd = jnp.where(causal, s[n - 128:], -1e30)
            mx = jnp.max(sd.reshape(16, 8, 128), axis=0)
            s_buf[OFF[j] + n - 128:OFF[j] + n, :] = sd
            if j > 0:
                s_buf[OFF[j]:OFF[j] + n - 128, :] = s[:n - 128]
                mx = jnp.maximum(mx, jnp.max(s[:n - 128].reshape(16 * j, 8, 128), axis=0))
            m_buf[j] = mx

    def pv(h, s_buf, m_buf):
        gm = gm_tab[pl.ds(DH * h, 24), :]
        for j in range(NT):
            n = 128 * (j + 1)
            m = jnp.max(m_buf[j], axis=0, keepdims=True)
            p = jnp.exp2(s_buf[OFF[j]:OFF[j] + n, :] - m).astype(bf16)
            vs = []
            for kb in range(j + 1):
                vv = v_buf[kb, pl.ds(9 * h, 16), :]
                vv = jnp.where(vrow == 9, jnp.uint32(ONE_LO), vv)
                vs.append(pltpu.bitcast(vv, bf16))
            va = jnp.concatenate(vs, axis=1) if j > 0 else vs[0]
            o = jnp.dot(va, p, preferred_element_type=f32)
            o = (o[:24] * gm) * (1.0 / o[18:19]) + am_buf[j, pl.ds(DH * h, 24), :]
            o_buf[j, pl.ds(DH * h, 24), :] = o

    def ln_in(s, j):
        ld = lambda c: xbuf[s, c * CH:(c + 1) * CH, j * 128:(j + 1) * 128].astype(f32)
        mean, rstd = _stats(ld(c) for c in range(D // CH))
        return jnp.concatenate([((ld(c) - mean) * rstd).astype(bf16) for c in range(D // CH)], axis=0)

    def proj_q(xn, j):
        t = jnp.dot(pltpu.bitcast(wall[0:NP // 2, :], bf16), xn, preferred_element_type=f32)
        for g in range(G):
            qg = t[GO[g]:GO[g] + GR[g]]
            q_buf[g, j, 0:GR[g] // 2, :] = pltpu.bitcast((qg * QSCALE).astype(bf16), u32)
            pq_buf[g, j, 0:GR[g] // 2, :] = pltpu.bitcast(_phi(qg).astype(bf16), u32)

    def proj_k(xn, j):
        t = jnp.dot(pltpu.bitcast(wall[NP // 2:NP, :], bf16), xn, preferred_element_type=f32)
        for g in range(G):
            kg = t[GO[g]:GO[g] + GR[g]]
            pk_buf[g, j, 0:GR[g] // 2, :] = pltpu.bitcast(_phi(kg).astype(bf16), u32)
            kb = kg.astype(bf16)
            if GR[g] < 128:
                kb = jnp.concatenate([kb, jnp.zeros((128 - GR[g], 128), bf16)], axis=0)
            k_buf[g, 64 * j:64 * (j + 1), :] = pltpu.bitcast(kb.T, u32)

    def proj_v(xn, j):
        t = jnp.dot(pltpu.bitcast(wall[NP:NP + D // 2, :], bf16), xn, preferred_element_type=f32)
        v_buf[j, 0:D // 2, :] = pltpu.bitcast(t.astype(bf16), u32)

    def retrieve():
        r8 = lax.broadcasted_iota(jnp.int32, (8, 128), 0)
        for g in range(G):
            mb = jnp.where(bd, m_st[g, 0:128, :], 0.0).astype(bf16)
            zb = jnp.where(zmask, m_st[g, 128:129, :], 0.0).astype(bf16)
            lhs = jnp.concatenate([mb[:GR[g]], zb], axis=0)
            for j in range(NT):
                rr = jnp.dot(lhs, pltpu.bitcast(pq_buf[g, j], bf16), preferred_element_type=f32)
                rd = 1.0 / (rr[GR[g]:GR[g] + 8] + 1e-6)
                rb = [jnp.broadcast_to(rd[i:i + 1], (8, 128)) for i in range(8)]
                for v in range(GR[g] // 8):
                    h1, h2 = (8 * v) // DH, (8 * v + 7) // DH
                    e = rb[h1] if h1 == h2 else jnp.where(r8 < h2 * DH - 8 * v, rb[h1], rb[h2])
                    gg = g_tab[g * GW + 8 * v:g * GW + 8 * v + 8, :]
                    am_buf[j, g * GW + 8 * v:g * GW + 8 * v + 8, :] = (gg * rr[8 * v:8 * v + 8]) * e

    def update():
        ones = jnp.ones((16, 128), bf16)
        for g in range(G):
            n = GR[g]
            acc = m_st[g]
            for kb in range(NT):
                vg = jnp.concatenate([pltpu.bitcast(v_buf[kb, g * 63:g * 63 + 64, :], bf16), ones], axis=0)
                acc = acc + lax.dot_general(vg, pltpu.bitcast(pk_buf[g, kb], bf16), _NT,
                                            preferred_element_type=f32)
            m_st[g] = acc

    def out_tile(s, j, rbest, ibest):
        att = jnp.dot(pltpu.bitcast(wo_t[...], bf16), o_buf[j, 0:D, :].astype(bf16), preferred_element_type=f32)
        t = s * NT + j

        def resid():
            for c in range(D // CH):
                rows = slice(c * CH, (c + 1) * CH)
                hh = xbuf[s, rows, j * 128:(j + 1) * 128].astype(f32) + att[rows]
                h_buf[t, rows, :] = hh
                yield hh
        mean, rstd = _stats(resid())
        racc = None
        for c in range(D // CH):
            rows = slice(c * CH, (c + 1) * CH)
            hh = h_buf[t, rows, :]
            ln = (hh - mean) * rstd
            obuf[s, rows, j * 128:(j + 1) * 128] = (hh + ln).astype(bf16)
            l_buf[t, rows, :] = ln.astype(bf16)
            racc = _fold(racc, ln * wr_tab[rows, :])
        r = jnp.sum(racc, axis=0, keepdims=True)
        take = r > rbest
        return jnp.where(take, r, rbest), jnp.where(take, lane + (s * L + j * 128), ibest)

    x_copy(0).wait()
    xns = [ln_in(0, j) for j in range(NT)]
    cp_wq.wait()
    put_padded(wq_v, 0)
    cp_wo.start(); x_copy(1).start()
    proj_q(xns[0], 0)
    cp_wk.wait()
    put_padded(wk_v, NP)
    for j in range(1, NT):
        proj_q(xns[j], j)
    cp_wv.wait()
    wall[NP:NP + D // 2, :] = pltpu.bitcast(wv_v[...].T, u32)
    x_copy(2).start(); x_copy(3).start()
    cp_wg.start(); cp_wu.start(); cp_wd.start()
    for j in range(NT):
        proj_k(xns[j], j)
    cp_wo.wait()
    wo_t[...] = pltpu.bitcast(wo_v[...].T, u32)
    for j in range(NT):
        proj_v(xns[j], j)
    qk(0, s0, m0)

    def segment(s, carry):
        def heads(i, c):
            for a in range(HU // 2):
                h = i * HU + 2 * a
                qk(h + 1, s1, m1)
                pv(h, s0, m0)
                qk(h + 2, s0, m0)
                pv(h + 1, s1, m1)
            return c
        lax.fori_loop(0, (H - 2) // HU, heads, 0)

        def mid(rbest, ibest):
            x_copy(s + 1).wait()
            qk(H - 1, s1, m1)
            pv(H - 2, s0, m0)
            update()
            xn = ln_in(s + 1, 0)
            proj_q(xn, 0)
            proj_k(xn, 0)
            pv(H - 1, s1, m1)
            proj_v(xn, 0)
            for j in range(NT):
                rbest, ibest = out_tile(s, j, rbest, ibest)
                if j + 1 < NT:
                    xn = ln_in(s + 1, j + 1)
                    proj_q(xn, j + 1)
                    proj_k(xn, j + 1)
                    proj_v(xn, j + 1)
            o_copy(s).start()
            retrieve()
            qk(0, s0, m0)
            return rbest, ibest

        def last(rbest, ibest):
            qk(H - 1, s1, m1)
            pv(H - 2, s0, m0)
            pv(H - 1, s1, m1)
            for j in range(NT):
                rbest, ibest = out_tile(s, j, rbest, ibest)
            o_copy(s).start()
            return rbest, ibest

        return lax.cond(s < NSEG - 1, mid, last, *carry)

    rbest, ibest = lax.fori_loop(
        0, NSEG, segment, (jnp.full((1, 128), -jnp.inf, f32), jnp.zeros((1, 128), jnp.int32)))

    rmax = jnp.max(rbest, axis=1, keepdims=True)
    imin = jnp.min(jnp.where(rbest == rmax, ibest.astype(f32), float(S)), axis=1, keepdims=True).astype(jnp.int32)
    tile = imin[0, 0] // 128
    onehot = lane == (imin & 127)
    oh = jnp.broadcast_to(jnp.where(onehot, 1.0, 0.0), (16, 128)).astype(bf16)
    xs = lax.dot_general(oh, l_buf[tile], _NT, preferred_element_type=f32).astype(bf16)
    hh = h_buf[tile]
    ln = _ln0(hh)
    cp_wg.wait(); cp_wu.wait(); cp_wd.wait()
    y = jnp.zeros((D, 128), f32)
    for c in range(F // FCH):
        cs = slice(c * FCH, (c + 1) * FCH)
        gt = jnp.dot(xs, wg_v[:, cs], preferred_element_type=f32)
        up = jnp.dot(xs, wu_v[:, cs], preferred_element_type=f32)
        act = (gt * jax.nn.sigmoid(gt) * up).astype(bf16).astype(f32)[0:1]
        pr = wd_v[:, cs].astype(f32) * act
        for cc in range(FCH // 128):
            y = y + pr[:, cc * 128:(cc + 1) * 128]
    y = jnp.sum(y, axis=1, keepdims=True) * jax.nn.sigmoid(rmax)
    new_tile = jnp.where(onehot, hh + (ln + y), hh + ln).astype(bf16)
    for s in range(NSEG):
        o_copy(s).wait()
    obuf[0, :, 0:128] = new_tile
    fin = pltpu.make_async_copy(obuf.at[0, :, 0:128],
                                out_hbm.at[0, :, pl.ds(pl.multiple_of(tile * 128, 128), 128)], sems.at[15])
    fin.start()
    fin.wait()


@jax.jit
def pallas_sequential_preLN__memory_aug_infini_attn__moe_arch_mod__prompt_kernel(
    A_x: jax.Array,
    A_wq: jax.Array,
    A_wk: jax.Array,
    A_wv: jax.Array,
    A_wo: jax.Array,
    A_beta: jax.Array,
    B_x: jax.Array,
    B_w_r: jax.Array,
    B_w_gate: jax.Array,
    B_w_up: jax.Array,
    B_w_down: jax.Array,
):
    hbm = pl.BlockSpec(memory_space=pltpu.HBM)
    vmem_spec = pl.BlockSpec(memory_space=pltpu.VMEM)
    V = pltpu.VMEM
    scratch = [
        V((NSEG, D, L), bf16),
        V((D, D), bf16), V((D, D), bf16), V((D, D), bf16), V((D, D), bf16),
        V((D, F), bf16), V((D, F), bf16), V((D, F), bf16),
        V((NP + D // 2, D), u32), V((D // 2, D), u32), V((D, 128), f32),
        V((G, L // 2, 128), u32), V((G, NT, 64, 128), u32),
        V((G, NT, 64, 128), u32), V((G, NT, 64, 128), u32),
        V((NT, 320, 128), u32),
        V((1280, 128), f32), V((1280, 128), f32), V((NT, 8, 128), f32), V((NT, 8, 128), f32),
        V((NT, 640, 128), f32), V((NT, 640, 128), f32), V((640, 128), f32), V((640, 128), f32),
        V((G, 144, 128), f32),
        V((S // 128, D, 128), f32), V((S // 128, D, 128), bf16), V((NSEG, D, L), bf16),
        pltpu.SemaphoreType.DMA((16,)),
    ]
    out_t = pl.pallas_call(
        _kernel,
        out_shape=jax.ShapeDtypeStruct((1, D, S), A_x.dtype),
        in_specs=[hbm] * 5 + [vmem_spec, vmem_spec] + [hbm] * 3,
        out_specs=hbm,
        scratch_shapes=scratch,
        compiler_params=pltpu.CompilerParams(vmem_limit_bytes=100 * 1024 * 1024),
    )(jnp.swapaxes(A_x, 1, 2), A_wq, A_wk, A_wv, A_wo, A_beta, B_w_r, B_w_gate, B_w_up, B_w_down.T)
    return jnp.swapaxes(out_t, 1, 2)
```

```python
import math

import jax
import jax.numpy as jnp
from jax import lax
import jax.experimental.pallas as pl
import jax.experimental.pallas.tpu as pltpu

bf16 = jnp.bfloat16
f32 = jnp.float32
u32 = jnp.uint32

S, D, H, DH, NSEG, L, F = 2048, 576, 32, 18, 4, 512, 4608
G = 5
GW = 126
GR = (128, 128, 128, 128, 80)
GO = (0, 128, 256, 384, 512)
NP = 592
NT = L // 128
OFF = (0, 128, 384, 768)
EPS = 1e-5
QSCALE = (DH ** -0.5) * math.log2(math.e)
ONE_LO = 0x00003F80
FCH = 512
HU = 10

_NT = (((1,), (1,)), ((), ()))


def _phi(t):
    return jnp.where(t > 0, t + 1.0, jnp.exp(t))


def _sum0(v):
    t = jnp.sum(v.reshape(8, D // 8, 128), axis=0)
    t = jnp.sum(t.reshape(3, D // 24, 128), axis=0)
    t = jnp.sum(t.reshape(3, 8, 128), axis=0)
    return jnp.sum(t, axis=0, keepdims=True)


CH = 48


def _fold(acc, c):
    t = jnp.sum(c.reshape(CH // 8, 8, 128), axis=0)
    return t if acc is None else acc + t


def _stats(chunks):
    s1 = s2 = shift = None
    for c in chunks:
        if shift is None:
            shift = c[0:1]
        d = c - shift
        s1 = _fold(s1, d)
        s2 = _fold(s2, d * d)
    m1 = jnp.sum(s1, axis=0, keepdims=True) * (1.0 / D)
    m2 = jnp.sum(s2, axis=0, keepdims=True) * (1.0 / D)
    var = jnp.maximum(m2 - m1 * m1, 0.0)
    return shift + m1, lax.rsqrt(var + EPS)


def _ln0(v):
    m = _sum0(v) * (1.0 / D)
    c = v - m
    var = _sum0(c * c) * (1.0 / D)
    return c * lax.rsqrt(var + EPS)


def _kernel(x_hbm, wq_hbm, wk_hbm, wv_hbm, wo_hbm, beta_ref, wr_ref, wg_hbm, wu_hbm, wd_hbm,
            out_hbm,
            xbuf, wq_v, wk_v, wv_v, wo_v, wg_v, wu_v, wd_v,
            wall, wo_t, wr_tab,
            k_buf, pk_buf, q_buf, pq_buf, v_buf,
            s0, s1, m0, m1, am_buf, o_buf, gm_tab, g_tab,
            m_st, h_buf, l_buf, obuf,
            sems):
    def x_copy(s):
        return pltpu.make_async_copy(x_hbm.at[0, :, pl.ds(s * L, L)], xbuf.at[s], sems.at[s])
    cp_wk = pltpu.make_async_copy(wk_hbm, wk_v, sems.at[4])
    cp_wq = pltpu.make_async_copy(wq_hbm, wq_v, sems.at[5])
    cp_wv = pltpu.make_async_copy(wv_hbm, wv_v, sems.at[6])
    cp_wo = pltpu.make_async_copy(wo_hbm, wo_v, sems.at[7])
    cp_wg = pltpu.make_async_copy(wg_hbm, wg_v, sems.at[8])
    cp_wu = pltpu.make_async_copy(wu_hbm, wu_v, sems.at[9])
    cp_wd = pltpu.make_async_copy(wd_hbm, wd_v, sems.at[10])

    def o_copy(s):
        return pltpu.make_async_copy(obuf.at[s], out_hbm.at[0, :, pl.ds(s * L, L)], sems.at[11 + s])

    x_copy(0).start(); cp_wq.start()

    gate = jax.nn.sigmoid(beta_ref[...].astype(f32).reshape(1, H))
    rowi = lax.broadcasted_iota(jnp.int32, (640, H), 0)
    coli = lax.broadcasted_iota(jnp.int32, (640, H), 1)
    gcol = jnp.sum(jnp.where((rowi >= coli * DH) & (rowi < coli * DH + DH), gate, 0.0), axis=1, keepdims=True)
    gfull = jnp.broadcast_to(gcol, (640, 128))
    gm_tab[...] = 1.0 - gfull
    g_tab[...] = gfull
    wr_tab[...] = jnp.broadcast_to(wr_ref[...].astype(f32).reshape(1, D), (128, D)).T
    am_buf[...] = jnp.zeros_like(am_buf)
    m_st[...] = jnp.zeros_like(m_st)
    o_buf[...] = jnp.zeros_like(o_buf)
    v_buf[...] = jnp.zeros_like(v_buf)
    pq_buf[...] = jnp.zeros_like(pq_buf)
    pk_buf[...] = jnp.zeros_like(pk_buf)
    k_buf[...] = jnp.zeros_like(k_buf)

    def put_padded(w_ref, base):
        wT = pltpu.bitcast(w_ref[...].T, u32)
        for g in range(G):
            w = min(GW, D - g * GW) // 2
            r0 = (base + GO[g]) // 2
            wall[r0:r0 + w, :] = wT[g * 63:g * 63 + w]
            wall[r0 + w:r0 + GR[g] // 2, :] = jnp.zeros((GR[g] // 2 - w, D), u32)

    row64 = lax.broadcasted_iota(jnp.int32, (64, 128), 0)
    vrow = lax.broadcasted_iota(jnp.int32, (16, 128), 0)
    kk = lax.broadcasted_iota(jnp.int32, (128, 128), 0)
    qq = lax.broadcasted_iota(jnp.int32, (128, 128), 1)
    causal = kk <= qq
    bd = jnp.zeros((128, 128), jnp.bool_)
    for r in range(7):
        bd = bd | ((kk >= r * DH) & (kk < r * DH + DH) & (qq >= r * DH) & (qq < r * DH + DH))
    lane = lax.broadcasted_iota(jnp.int32, (1, 128), 1)
    zr = lax.broadcasted_iota(jnp.int32, (16, 128), 0)
    zc = lax.broadcasted_iota(jnp.int32, (16, 128), 1)
    zmask = (zc >= zr * DH) & (zc < zr * DH + DH)

    def qk(h, s_buf, m_buf):
        g = h // 7
        r = h - g * 7
        qmask = (row64 >= 9 * r) & (row64 < 9 * r + 9)
        for j in reversed(range(NT)):
            n = 128 * (j + 1)
            qt = pltpu.bitcast(jnp.where(qmask, q_buf[g, j], jnp.uint32(0)), bf16)
            kt = pltpu.bitcast(k_buf[g, 0:n // 2, :], bf16)
            s = jnp.dot(kt, qt, preferred_element_type=f32)
            sd = jnp.where(causal, s[n - 128:], -1e30)
            mx = jnp.max(sd.reshape(16, 8, 128), axis=0)
            s_buf[OFF[j] + n - 128:OFF[j] + n, :] = sd
            if j > 0:
                s_buf[OFF[j]:OFF[j] + n - 128, :] = s[:n - 128]
                mx = jnp.maximum(mx, jnp.max(s[:n - 128].reshape(16 * j, 8, 128), axis=0))
            m_buf[j] = mx

    def pv(h, s_buf, m_buf):
        gm = gm_tab[pl.ds(DH * h, 24), :]
        for j in range(NT):
            n = 128 * (j + 1)
            m = jnp.max(m_buf[j], axis=0, keepdims=True)
            p = jnp.exp2(s_buf[OFF[j]:OFF[j] + n, :] - m).astype(bf16)
            vs = []
            for kb in range(j + 1):
                vv = v_buf[kb, pl.ds(9 * h, 16), :]
                vv = jnp.where(vrow == 9, jnp.uint32(ONE_LO), vv)
                vs.append(pltpu.bitcast(vv, bf16))
            va = jnp.concatenate(vs, axis=1) if j > 0 else vs[0]
            o = jnp.dot(va, p, preferred_element_type=f32)
            o = (o[:24] * gm) * (1.0 / o[18:19]) + am_buf[j, pl.ds(DH * h, 24), :]
            o_buf[j, pl.ds(DH * h, 24), :] = o

    def ln_in(s, j):
        ld = lambda c: xbuf[s, c * CH:(c + 1) * CH, j * 128:(j + 1) * 128].astype(f32)
        mean, rstd = _stats(ld(c) for c in range(D // CH))
        return jnp.concatenate([((ld(c) - mean) * rstd).astype(bf16) for c in range(D // CH)], axis=0)

    def proj_q(xn, j):
        t = jnp.dot(pltpu.bitcast(wall[0:NP // 2, :], bf16), xn, preferred_element_type=f32)
        for g in range(G):
            qg = t[GO[g]:GO[g] + GR[g]]
            q_buf[g, j, 0:GR[g] // 2, :] = pltpu.bitcast((qg * QSCALE).astype(bf16), u32)
            pq_buf[g, j, 0:GR[g] // 2, :] = pltpu.bitcast(_phi(qg).astype(bf16), u32)

    def proj_k(xn, j):
        t = jnp.dot(pltpu.bitcast(wall[NP // 2:NP, :], bf16), xn, preferred_element_type=f32)
        for g in range(G):
            kg = t[GO[g]:GO[g] + GR[g]]
            pk_buf[g, j, 0:GR[g] // 2, :] = pltpu.bitcast(_phi(kg).astype(bf16), u32)
            kb = kg.astype(bf16)
            if GR[g] < 128:
                kb = jnp.concatenate([kb, jnp.zeros((128 - GR[g], 128), bf16)], axis=0)
            k_buf[g, 64 * j:64 * (j + 1), :] = pltpu.bitcast(kb.T, u32)

    def proj_v(xn, j):
        t = jnp.dot(pltpu.bitcast(wall[NP:NP + D // 2, :], bf16), xn, preferred_element_type=f32)
        v_buf[j, 0:D // 2, :] = pltpu.bitcast(t.astype(bf16), u32)

    def retrieve():
        r8 = lax.broadcasted_iota(jnp.int32, (8, 128), 0)
        for g in range(G):
            mb = jnp.where(bd, m_st[g, 0:128, :], 0.0).astype(bf16)
            zb = jnp.where(zmask, m_st[g, 128:129, :], 0.0).astype(bf16)
            lhs = jnp.concatenate([mb[:GR[g]], zb], axis=0)
            for j in range(NT):
                rr = jnp.dot(lhs, pltpu.bitcast(pq_buf[g, j], bf16), preferred_element_type=f32)
                rd = 1.0 / (rr[GR[g]:GR[g] + 8] + 1e-6)
                rb = [jnp.broadcast_to(rd[i:i + 1], (8, 128)) for i in range(8)]
                for v in range(GR[g] // 8):
                    h1, h2 = (8 * v) // DH, (8 * v + 7) // DH
                    e = rb[h1] if h1 == h2 else jnp.where(r8 < h2 * DH - 8 * v, rb[h1], rb[h2])
                    gg = g_tab[g * GW + 8 * v:g * GW + 8 * v + 8, :]
                    am_buf[j, g * GW + 8 * v:g * GW + 8 * v + 8, :] = (gg * rr[8 * v:8 * v + 8]) * e

    def update():
        ones = jnp.ones((16, 128), bf16)
        for g in range(G):
            n = GR[g]
            acc = m_st[g]
            for kb in range(NT):
                vg = jnp.concatenate([pltpu.bitcast(v_buf[kb, g * 63:g * 63 + 64, :], bf16), ones], axis=0)
                acc = acc + lax.dot_general(vg, pltpu.bitcast(pk_buf[g, kb], bf16), _NT,
                                            preferred_element_type=f32)
            m_st[g] = acc

    def out_tile(s, j, rbest, ibest):
        att = jnp.dot(pltpu.bitcast(wo_t[...], bf16), o_buf[j, 0:D, :].astype(bf16), preferred_element_type=f32)
        t = s * NT + j

        def resid():
            for c in range(D // CH):
                rows = slice(c * CH, (c + 1) * CH)
                hh = xbuf[s, rows, j * 128:(j + 1) * 128].astype(f32) + att[rows]
                h_buf[t, rows, :] = hh
                yield hh
        mean, rstd = _stats(resid())
        racc = None
        for c in range(D // CH):
            rows = slice(c * CH, (c + 1) * CH)
            hh = h_buf[t, rows, :]
            ln = (hh - mean) * rstd
            obuf[s, rows, j * 128:(j + 1) * 128] = (hh + ln).astype(bf16)
            l_buf[t, rows, :] = ln.astype(bf16)
            racc = _fold(racc, ln * wr_tab[rows, :])
        r = jnp.sum(racc, axis=0, keepdims=True)
        take = r > rbest
        return jnp.where(take, r, rbest), jnp.where(take, lane + (s * L + j * 128), ibest)

    x_copy(0).wait()
    cp_wq.wait()
    cp_wk.start(); cp_wv.start(); cp_wo.start(); x_copy(1).start()
    xns = [ln_in(0, j) for j in range(NT)]
    put_padded(wq_v, 0)
    proj_q(xns[0], 0)
    proj_q(xns[1], 1)
    cp_wk.wait(); cp_wv.wait()
    x_copy(2).start(); x_copy(3).start()
    cp_wg.start(); cp_wu.start(); cp_wd.start()
    proj_q(xns[2], 2)
    put_padded(wk_v, NP)
    proj_q(xns[3], 3)
    wall[NP:NP + D // 2, :] = pltpu.bitcast(wv_v[...].T, u32)
    for j in range(NT):
        proj_k(xns[j], j)
    proj_v(xns[0], 0)
    cp_wo.wait()
    for j in range(1, NT):
        proj_v(xns[j], j)
    wo_t[...] = pltpu.bitcast(wo_v[...].T, u32)
    qk(0, s0, m0)

    def segment(s, carry):
        def heads(i, c):
            for a in range(HU // 2):
                h = i * HU + 2 * a
                qk(h + 1, s1, m1)
                pv(h, s0, m0)
                qk(h + 2, s0, m0)
                pv(h + 1, s1, m1)
            return c
        lax.fori_loop(0, (H - 2) // HU, heads, 0)

        def mid(rbest, ibest):
            x_copy(s + 1).wait()
            qk(H - 1, s1, m1)
            pv(H - 2, s0, m0)
            update()
            xn = ln_in(s + 1, 0)
            proj_q(xn, 0)
            proj_k(xn, 0)
            pv(H - 1, s1, m1)
            proj_v(xn, 0)
            for j in range(NT):
                rbest, ibest = out_tile(s, j, rbest, ibest)
                if j + 1 < NT:
                    xn = ln_in(s + 1, j + 1)
                    proj_q(xn, j + 1)
                    proj_k(xn, j + 1)
                    proj_v(xn, j + 1)
            o_copy(s).start()
            retrieve()
            qk(0, s0, m0)
            return rbest, ibest

        def last(rbest, ibest):
            qk(H - 1, s1, m1)
            pv(H - 2, s0, m0)
            pv(H - 1, s1, m1)
            for j in range(NT):
                rbest, ibest = out_tile(s, j, rbest, ibest)
            o_copy(s).start()
            return rbest, ibest

        return lax.cond(s < NSEG - 1, mid, last, *carry)

    rbest, ibest = lax.fori_loop(
        0, NSEG, segment, (jnp.full((1, 128), -jnp.inf, f32), jnp.zeros((1, 128), jnp.int32)))

    rmax = jnp.max(rbest, axis=1, keepdims=True)
    imin = jnp.min(jnp.where(rbest == rmax, ibest.astype(f32), float(S)), axis=1, keepdims=True).astype(jnp.int32)
    tile = imin[0, 0] // 128
    onehot = lane == (imin & 127)
    oh = jnp.broadcast_to(jnp.where(onehot, 1.0, 0.0), (16, 128)).astype(bf16)
    xs = lax.dot_general(oh, l_buf[tile], _NT, preferred_element_type=f32).astype(bf16)
    hh = h_buf[tile]
    ln = _ln0(hh)
    cp_wg.wait(); cp_wu.wait(); cp_wd.wait()
    y = jnp.zeros((D, 128), f32)
    for c in range(F // FCH):
        cs = slice(c * FCH, (c + 1) * FCH)
        gt = jnp.dot(xs, wg_v[:, cs], preferred_element_type=f32)
        up = jnp.dot(xs, wu_v[:, cs], preferred_element_type=f32)
        act = (gt * jax.nn.sigmoid(gt) * up).astype(bf16).astype(f32)[0:1]
        pr = wd_v[:, cs].astype(f32) * act
        for cc in range(FCH // 128):
            y = y + pr[:, cc * 128:(cc + 1) * 128]
    y = jnp.sum(y, axis=1, keepdims=True) * jax.nn.sigmoid(rmax)
    new_tile = jnp.where(onehot, hh + (ln + y), hh + ln).astype(bf16)
    for s in range(NSEG):
        o_copy(s).wait()
    obuf[0, :, 0:128] = new_tile
    fin = pltpu.make_async_copy(obuf.at[0, :, 0:128],
                                out_hbm.at[0, :, pl.ds(pl.multiple_of(tile * 128, 128), 128)], sems.at[15])
    fin.start()
    fin.wait()


@jax.jit
def pallas_sequential_preLN__memory_aug_infini_attn__moe_arch_mod__prompt_kernel(
    A_x: jax.Array,
    A_wq: jax.Array,
    A_wk: jax.Array,
    A_wv: jax.Array,
    A_wo: jax.Array,
    A_beta: jax.Array,
    B_x: jax.Array,
    B_w_r: jax.Array,
    B_w_gate: jax.Array,
    B_w_up: jax.Array,
    B_w_down: jax.Array,
):
    hbm = pl.BlockSpec(memory_space=pltpu.HBM)
    vmem_spec = pl.BlockSpec(memory_space=pltpu.VMEM)
    V = pltpu.VMEM
    scratch = [
        V((NSEG, D, L), bf16),
        V((D, D), bf16), V((D, D), bf16), V((D, D), bf16), V((D, D), bf16),
        V((D, F), bf16), V((D, F), bf16), V((D, F), bf16),
        V((NP + D // 2, D), u32), V((D // 2, D), u32), V((D, 128), f32),
        V((G, L // 2, 128), u32), V((G, NT, 64, 128), u32),
        V((G, NT, 64, 128), u32), V((G, NT, 64, 128), u32),
        V((NT, 320, 128), u32),
        V((1280, 128), f32), V((1280, 128), f32), V((NT, 8, 128), f32), V((NT, 8, 128), f32),
        V((NT, 640, 128), f32), V((NT, 640, 128), f32), V((640, 128), f32), V((640, 128), f32),
        V((G, 144, 128), f32),
        V((S // 128, D, 128), f32), V((S // 128, D, 128), bf16), V((NSEG, D, L), bf16),
        pltpu.SemaphoreType.DMA((16,)),
    ]
    out_t = pl.pallas_call(
        _kernel,
        out_shape=jax.ShapeDtypeStruct((1, D, S), A_x.dtype),
        in_specs=[hbm] * 5 + [vmem_spec, vmem_spec] + [hbm] * 3,
        out_specs=hbm,
        scratch_shapes=scratch,
        compiler_params=pltpu.CompilerParams(vmem_limit_bytes=100 * 1024 * 1024),
    )(jnp.swapaxes(A_x, 1, 2), A_wq, A_wk, A_wv, A_wo, A_beta, B_w_r, B_w_gate, B_w_up, B_w_down.T)
    return jnp.swapaxes(out_t, 1, 2)
```

```python
import math

import jax
import jax.numpy as jnp
from jax import lax
import jax.experimental.pallas as pl
import jax.experimental.pallas.tpu as pltpu

bf16 = jnp.bfloat16
f32 = jnp.float32
u32 = jnp.uint32

S, D, H, DH, NSEG, L, F = 2048, 576, 32, 18, 4, 512, 4608
G = 5
GW = 126
GR = (128, 128, 128, 128, 80)
GO = (0, 128, 256, 384, 512)
NP = 592
NT = L // 128
OFF = (0, 128, 384, 768)
EPS = 1e-5
QSCALE = (DH ** -0.5) * math.log2(math.e)
ONE_LO = 0x00003F80
FP = 6
HU = 10

_NT = (((1,), (1,)), ((), ()))


def _phi(t):
    return jnp.where(t > 0, t + 1.0, jnp.exp(t))


def _sum0(v):
    t = jnp.sum(v.reshape(8, D // 8, 128), axis=0)
    t = jnp.sum(t.reshape(3, D // 24, 128), axis=0)
    t = jnp.sum(t.reshape(3, 8, 128), axis=0)
    return jnp.sum(t, axis=0, keepdims=True)


CH = 48


def _fold(acc, c):
    t = jnp.sum(c.reshape(CH // 8, 8, 128), axis=0)
    return t if acc is None else acc + t


def _stats(chunks):
    s1 = s2 = shift = None
    for c in chunks:
        if shift is None:
            shift = c[0:1]
        d = c - shift
        s1 = _fold(s1, d)
        s2 = _fold(s2, d * d)
    m1 = jnp.sum(s1, axis=0, keepdims=True) * (1.0 / D)
    m2 = jnp.sum(s2, axis=0, keepdims=True) * (1.0 / D)
    var = jnp.maximum(m2 - m1 * m1, 0.0)
    return shift + m1, lax.rsqrt(var + EPS)


def _ln0(v):
    m = _sum0(v) * (1.0 / D)
    c = v - m
    var = _sum0(c * c) * (1.0 / D)
    return c * lax.rsqrt(var + EPS)


def _kernel(x_hbm, wq_hbm, wk_hbm, wv_hbm, wo_hbm, beta_ref, wr_ref, wg_hbm, wu_hbm, wd_hbm,
            out_hbm,
            xbuf, wq_v, wk_v, wv_v, wo_v, wg_v, wu_v, wd_v,
            wall, wo_t, wr_tab,
            k_buf, pk_buf, q_buf, pq_buf, v_buf,
            s0, s1, m0, m1, am_buf, o_buf, gm_tab, g_tab,
            m_st, h_buf, l_buf, obuf,
            sems):
    def x_copy(s):
        return pltpu.make_async_copy(x_hbm.at[0, :, pl.ds(s * L, L)], xbuf.at[s], sems.at[s])
    cp_wk = pltpu.make_async_copy(wk_hbm, wk_v, sems.at[4])
    cp_wq = pltpu.make_async_copy(wq_hbm, wq_v, sems.at[5])
    cp_wv = pltpu.make_async_copy(wv_hbm, wv_v, sems.at[6])
    cp_wo = pltpu.make_async_copy(wo_hbm, wo_v, sems.at[7])
    cp_gu = [pltpu.make_async_copy(src.at[:, pl.ds(c * 128, 128)], dst.at[c], sems.at[k])
             for src, dst, k in ((wg_hbm, wg_v, 8), (wu_hbm, wu_v, 9)) for c in range(F // 128)]
    cp_wd = pltpu.make_async_copy(wd_hbm, wd_v, sems.at[10])

    def o_copy(s):
        return pltpu.make_async_copy(obuf.at[s], out_hbm.at[0, :, pl.ds(s * L, L)], sems.at[11 + s])

    def x0_copy(i):
        return pltpu.make_async_copy(x_hbm.at[0, :, pl.ds(i * 256, 256)], xbuf.at[0, :, pl.ds(i * 256, 256)],
                                     sems.at[16 * i])

    x0_copy(0).start(); cp_wq.start(); x0_copy(1).start()

    gate = jax.nn.sigmoid(beta_ref[...].astype(f32).reshape(1, H))
    rowi = lax.broadcasted_iota(jnp.int32, (640, H), 0)
    coli = lax.broadcasted_iota(jnp.int32, (640, H), 1)
    gcol = jnp.sum(jnp.where((rowi >= coli * DH) & (rowi < coli * DH + DH), gate, 0.0), axis=1, keepdims=True)
    gfull = jnp.broadcast_to(gcol, (640, 128))
    gm_tab[...] = 1.0 - gfull
    g_tab[...] = gfull
    wr_tab[...] = jnp.broadcast_to(wr_ref[...].astype(f32).reshape(1, D), (128, D)).T
    am_buf[...] = jnp.zeros_like(am_buf)
    m_st[...] = jnp.zeros_like(m_st)
    o_buf[...] = jnp.zeros_like(o_buf)
    v_buf[...] = jnp.zeros_like(v_buf)
    pq_buf[...] = jnp.zeros_like(pq_buf)
    pk_buf[...] = jnp.zeros_like(pk_buf)
    k_buf[...] = jnp.zeros_like(k_buf)

    def put_padded(w_ref, base):
        wT = pltpu.bitcast(w_ref[...].T, u32)
        for g in range(G):
            w = min(GW, D - g * GW) // 2
            r0 = (base + GO[g]) // 2
            wall[r0:r0 + w, :] = wT[g * 63:g * 63 + w]
            wall[r0 + w:r0 + GR[g] // 2, :] = jnp.zeros((GR[g] // 2 - w, D), u32)

    row64 = lax.broadcasted_iota(jnp.int32, (64, 128), 0)
    vrow = lax.broadcasted_iota(jnp.int32, (16, 128), 0)
    kk = lax.broadcasted_iota(jnp.int32, (128, 128), 0)
    qq = lax.broadcasted_iota(jnp.int32, (128, 128), 1)
    causal = kk <= qq
    bd = jnp.zeros((128, 128), jnp.bool_)
    for r in range(7):
        bd = bd | ((kk >= r * DH) & (kk < r * DH + DH) & (qq >= r * DH) & (qq < r * DH + DH))
    lane = lax.broadcasted_iota(jnp.int32, (1, 128), 1)
    zr = lax.broadcasted_iota(jnp.int32, (16, 128), 0)
    zc = lax.broadcasted_iota(jnp.int32, (16, 128), 1)
    zmask = (zc >= zr * DH) & (zc < zr * DH + DH)

    def qk(h, s_buf, m_buf):
        g = h // 7
        r = h - g * 7
        qmask = (row64 >= 9 * r) & (row64 < 9 * r + 9)
        for j in reversed(range(NT)):
            n = 128 * (j + 1)
            qt = pltpu.bitcast(jnp.where(qmask, q_buf[g, j], jnp.uint32(0)), bf16)
            kt = pltpu.bitcast(k_buf[g, 0:n // 2, :], bf16)
            s = jnp.dot(kt, qt, preferred_element_type=f32)
            sd = jnp.where(causal, s[n - 128:], -1e30)
            mx = jnp.max(sd.reshape(16, 8, 128), axis=0)
            s_buf[OFF[j] + n - 128:OFF[j] + n, :] = sd
            if j > 0:
                s_buf[OFF[j]:OFF[j] + n - 128, :] = s[:n - 128]
                mx = jnp.maximum(mx, jnp.max(s[:n - 128].reshape(16 * j, 8, 128), axis=0))
            m_buf[j] = mx

    def pv(h, s_buf, m_buf):
        gm = gm_tab[pl.ds(DH * h, 24), :]
        for j in range(NT):
            n = 128 * (j + 1)
            m = jnp.max(m_buf[j], axis=0, keepdims=True)
            p = jnp.exp2(s_buf[OFF[j]:OFF[j] + n, :] - m).astype(bf16)
            vs = []
            for kb in range(j + 1):
                vv = v_buf[kb, pl.ds(9 * h, 16), :]
                vv = jnp.where(vrow == 9, jnp.uint32(ONE_LO), vv)
                vs.append(pltpu.bitcast(vv, bf16))
            va = jnp.concatenate(vs, axis=1) if j > 0 else vs[0]
            o = jnp.dot(va, p, preferred_element_type=f32)
            o = (o[:24] * gm) * (1.0 / o[18:19]) + am_buf[j, pl.ds(DH * h, 24), :]
            o_buf[j, pl.ds(DH * h, 24), :] = o

    def ln_in(s, j):
        ld = lambda c: xbuf[s, c * CH:(c + 1) * CH, j * 128:(j + 1) * 128].astype(f32)
        mean, rstd = _stats(ld(c) for c in range(D // CH))
        return jnp.concatenate([((ld(c) - mean) * rstd).astype(bf16) for c in range(D // CH)], axis=0)

    def proj_q(xn, j):
        t = jnp.dot(pltpu.bitcast(wall[0:NP // 2, :], bf16), xn, preferred_element_type=f32)
        for g in range(G):
            qg = t[GO[g]:GO[g] + GR[g]]
            q_buf[g, j, 0:GR[g] // 2, :] = pltpu.bitcast((qg * QSCALE).astype(bf16), u32)
            pq_buf[g, j, 0:GR[g] // 2, :] = pltpu.bitcast(_phi(qg).astype(bf16), u32)

    def proj_k(xn, j):
        t = jnp.dot(pltpu.bitcast(wall[NP // 2:NP, :], bf16), xn, preferred_element_type=f32)
        for g in range(G):
            kg = t[GO[g]:GO[g] + GR[g]]
            pk_buf[g, j, 0:GR[g] // 2, :] = pltpu.bitcast(_phi(kg).astype(bf16), u32)
            kb = kg.astype(bf16)
            if GR[g] < 128:
                kb = jnp.concatenate([kb, jnp.zeros((128 - GR[g], 128), bf16)], axis=0)
            k_buf[g, 64 * j:64 * (j + 1), :] = pltpu.bitcast(kb.T, u32)

    def proj_v(xn, j):
        t = jnp.dot(pltpu.bitcast(wall[NP:NP + D // 2, :], bf16), xn, preferred_element_type=f32)
        v_buf[j, 0:D // 2, :] = pltpu.bitcast(t.astype(bf16), u32)

    def retrieve():
        r8 = lax.broadcasted_iota(jnp.int32, (8, 128), 0)
        for g in range(G):
            mb = jnp.where(bd, m_st[g, 0:128, :], 0.0).astype(bf16)
            zb = jnp.where(zmask, m_st[g, 128:129, :], 0.0).astype(bf16)
            lhs = jnp.concatenate([mb[:GR[g]], zb], axis=0)
            for j in range(NT):
                rr = jnp.dot(lhs, pltpu.bitcast(pq_buf[g, j], bf16), preferred_element_type=f32)
                rd = 1.0 / (rr[GR[g]:GR[g] + 8] + 1e-6)
                rb = [jnp.broadcast_to(rd[i:i + 1], (8, 128)) for i in range(8)]
                for v in range(GR[g] // 8):
                    h1, h2 = (8 * v) // DH, (8 * v + 7) // DH
                    e = rb[h1] if h1 == h2 else jnp.where(r8 < h2 * DH - 8 * v, rb[h1], rb[h2])
                    gg = g_tab[g * GW + 8 * v:g * GW + 8 * v + 8, :]
                    am_buf[j, g * GW + 8 * v:g * GW + 8 * v + 8, :] = (gg * rr[8 * v:8 * v + 8]) * e

    def update():
        ones = jnp.ones((16, 128), bf16)
        for g in range(G):
            n = GR[g]
            acc = m_st[g]
            for kb in range(NT):
                vg = jnp.concatenate([pltpu.bitcast(v_buf[kb, g * 63:g * 63 + 64, :], bf16), ones], axis=0)
                acc = acc + lax.dot_general(vg, pltpu.bitcast(pk_buf[g, kb], bf16), _NT,
                                            preferred_element_type=f32)
            m_st[g] = acc

    def out_tile(s, j, rbest, ibest):
        att = jnp.dot(pltpu.bitcast(wo_t[...], bf16), o_buf[j, 0:D, :].astype(bf16), preferred_element_type=f32)
        t = s * NT + j

        def resid():
            for c in range(D // CH):
                rows = slice(c * CH, (c + 1) * CH)
                hh = xbuf[s, rows, j * 128:(j + 1) * 128].astype(f32) + att[rows]
                h_buf[t, rows, :] = hh
                yield hh
        mean, rstd = _stats(resid())
        racc = None
        for c in range(D // CH):
            rows = slice(c * CH, (c + 1) * CH)
            hh = h_buf[t, rows, :]
            ln = (hh - mean) * rstd
            obuf[s, rows, j * 128:(j + 1) * 128] = (hh + ln).astype(bf16)
            l_buf[t, rows, :] = ln.astype(bf16)
            racc = _fold(racc, ln * wr_tab[rows, :])
        r = jnp.sum(racc, axis=0, keepdims=True)
        take = r > rbest
        return jnp.where(take, r, rbest), jnp.where(take, lane + (s * L + j * 128), ibest)

    x0_copy(0).wait()
    cp_wq.wait()
    cp_wk.start(); cp_wv.start(); cp_wo.start(); x_copy(1).start()
    xns = [ln_in(0, j) for j in range(2)]
    put_padded(wq_v, 0)
    proj_q(xns[0], 0)
    x0_copy(1).wait()
    xns += [ln_in(0, j) for j in range(2, NT)]
    proj_q(xns[1], 1)
    proj_q(xns[2], 2)
    cp_wk.wait(); cp_wv.wait()
    x_copy(2).start(); x_copy(3).start()
    for cp in cp_gu:
        cp.start()
    cp_wd.start()
    proj_q(xns[3], 3)
    put_padded(wk_v, NP)
    wall[NP:NP + D // 2, :] = pltpu.bitcast(wv_v[...].T, u32)
    for j in range(NT):
        proj_k(xns[j], j)
    proj_v(xns[0], 0)
    cp_wo.wait()
    for j in range(1, NT):
        proj_v(xns[j], j)
    wo_t[...] = pltpu.bitcast(wo_v[...].T, u32)
    qk(0, s0, m0)

    def segment(s, carry):
        def heads(i, c):
            for a in range(HU // 2):
                h = i * HU + 2 * a
                qk(h + 1, s1, m1)
                pv(h, s0, m0)
                qk(h + 2, s0, m0)
                pv(h + 1, s1, m1)
            return c
        lax.fori_loop(0, (H - 2) // HU, heads, 0)

        def mid(rbest, ibest):
            x_copy(s + 1).wait()
            qk(H - 1, s1, m1)
            pv(H - 2, s0, m0)
            update()
            xn = ln_in(s + 1, 0)
            proj_q(xn, 0)
            proj_k(xn, 0)
            pv(H - 1, s1, m1)
            proj_v(xn, 0)
            for j in range(NT):
                rbest, ibest = out_tile(s, j, rbest, ibest)
                if j + 1 < NT:
                    xn = ln_in(s + 1, j + 1)
                    proj_q(xn, j + 1)
                    proj_k(xn, j + 1)
                    proj_v(xn, j + 1)
            o_copy(s).start()
            retrieve()
            qk(0, s0, m0)
            return rbest, ibest

        def last(rbest, ibest):
            qk(H - 1, s1, m1)
            pv(H - 2, s0, m0)
            pv(H - 1, s1, m1)
            for j in range(NT):
                rbest, ibest = out_tile(s, j, rbest, ibest)
            o_copy(s).start()
            return rbest, ibest

        return lax.cond(s < NSEG - 1, mid, last, *carry)

    rbest, ibest = lax.fori_loop(
        0, NSEG, segment, (jnp.full((1, 128), -jnp.inf, f32), jnp.zeros((1, 128), jnp.int32)))

    rmax = jnp.max(rbest, axis=1, keepdims=True)
    imin = jnp.min(jnp.where(rbest == rmax, ibest.astype(f32), float(S)), axis=1, keepdims=True).astype(jnp.int32)
    tile = imin[0, 0] // 128
    onehot = lane == (imin & 127)
    oh = jnp.broadcast_to(jnp.where(onehot, 1.0, 0.0), (16, 128)).astype(bf16)
    xs = lax.dot_general(oh, l_buf[tile], _NT, preferred_element_type=f32).astype(bf16)
    hh = h_buf[tile]
    ln = _ln0(hh)
    for cp in cp_gu:
        cp.wait()
    cp_wd.wait()
    wg32, wu32 = wg_v.bitcast(u32), wu_v.bitcast(u32)

    def gate_up(ph):
        acts = []
        for c in range(ph * FP, (ph + 1) * FP):
            gt = jnp.dot(xs, pltpu.bitcast(wg32[c], bf16), preferred_element_type=f32)[0:8]
            up = jnp.dot(xs, pltpu.bitcast(wu32[c], bf16), preferred_element_type=f32)[0:8]
            acts.append((gt * jax.nn.sigmoid(gt) * up).astype(bf16).astype(f32))
        return acts

    def down(ph, acts):
        for r in range(D // 16):
            rows = slice(r * 16, (r + 1) * 16)
            acc = None
            for i, c in enumerate(range(ph * FP, (ph + 1) * FP)):
                pr = wd_v[rows, c * 128:(c + 1) * 128].astype(f32).reshape(2, 8, 128) * acts[i]
                acc = pr if acc is None else acc + pr
            acc = acc.reshape(16, 128)
            wr_tab[rows, :] = acc if ph == 0 else wr_tab[rows, :] + acc

    acts = gate_up(0)
    for ph in range(F // 128 // FP):
        nxt = gate_up(ph + 1) if (ph + 1) * FP < F // 128 else None
        down(ph, acts)
        acts = nxt
    y = wr_tab[...]
    y = jnp.sum(y, axis=1, keepdims=True) * jax.nn.sigmoid(rmax)
    new_tile = jnp.where(onehot, hh + (ln + y), hh + ln).astype(bf16)
    for s in range(NSEG):
        o_copy(s).wait()
    obuf[0, :, 0:128] = new_tile
    fin = pltpu.make_async_copy(obuf.at[0, :, 0:128],
                                out_hbm.at[0, :, pl.ds(pl.multiple_of(tile * 128, 128), 128)], sems.at[15])
    fin.start()
    fin.wait()


@jax.jit
def pallas_sequential_preLN__memory_aug_infini_attn__moe_arch_mod__prompt_kernel(
    A_x: jax.Array,
    A_wq: jax.Array,
    A_wk: jax.Array,
    A_wv: jax.Array,
    A_wo: jax.Array,
    A_beta: jax.Array,
    B_x: jax.Array,
    B_w_r: jax.Array,
    B_w_gate: jax.Array,
    B_w_up: jax.Array,
    B_w_down: jax.Array,
):
    hbm = pl.BlockSpec(memory_space=pltpu.HBM)
    vmem_spec = pl.BlockSpec(memory_space=pltpu.VMEM)
    V = pltpu.VMEM
    scratch = [
        V((NSEG, D, L), bf16),
        V((D, D), bf16), V((D, D), bf16), V((D, D), bf16), V((D, D), bf16),
        V((F // 128, D, 128), bf16), V((F // 128, D, 128), bf16), V((D, F), bf16),
        V((NP + D // 2, D), u32), V((D // 2, D), u32), V((D, 128), f32),
        V((G, L // 2, 128), u32), V((G, NT, 64, 128), u32),
        V((G, NT, 64, 128), u32), V((G, NT, 64, 128), u32),
        V((NT, 320, 128), u32),
        V((1280, 128), f32), V((1280, 128), f32), V((NT, 8, 128), f32), V((NT, 8, 128), f32),
        V((NT, 640, 128), f32), V((NT, 640, 128), f32), V((640, 128), f32), V((640, 128), f32),
        V((G, 144, 128), f32),
        V((S // 128, D, 128), f32), V((S // 128, D, 128), bf16), V((NSEG, D, L), bf16),
        pltpu.SemaphoreType.DMA((17,)),
    ]
    out_t = pl.pallas_call(
        _kernel,
        out_shape=jax.ShapeDtypeStruct((1, D, S), A_x.dtype),
        in_specs=[hbm] * 5 + [vmem_spec, vmem_spec] + [hbm] * 3,
        out_specs=hbm,
        scratch_shapes=scratch,
        compiler_params=pltpu.CompilerParams(vmem_limit_bytes=100 * 1024 * 1024),
    )(jnp.swapaxes(A_x, 1, 2), A_wq, A_wk, A_wv, A_wo, A_beta, B_w_r, B_w_gate, B_w_up, B_w_down.T)
    return jnp.swapaxes(out_t, 1, 2)
```

```python
import math

import jax
import jax.numpy as jnp
from jax import lax
import jax.experimental.pallas as pl
import jax.experimental.pallas.tpu as pltpu

bf16 = jnp.bfloat16
f32 = jnp.float32
u32 = jnp.uint32

S, D, H, DH, NSEG, L, F = 2048, 576, 32, 18, 4, 512, 4608
G = 5
GW = 126
GR = (128, 128, 128, 128, 80)
GO = (0, 128, 256, 384, 512)
NP = 592
NT = L // 128
OFF = (0, 128, 384, 768)
EPS = 1e-5
QSCALE = (DH ** -0.5) * math.log2(math.e)
ONE_LO = 0x00003F80
FCH = 512
HU = 10

_NT = (((1,), (1,)), ((), ()))


def _phi(t):
    return jnp.where(t > 0, t + 1.0, jnp.exp(t))


def _sum0(v):
    t = jnp.sum(v.reshape(8, D // 8, 128), axis=0)
    t = jnp.sum(t.reshape(3, D // 24, 128), axis=0)
    t = jnp.sum(t.reshape(3, 8, 128), axis=0)
    return jnp.sum(t, axis=0, keepdims=True)


CH = 48


def _fold(acc, c):
    t = jnp.sum(c.reshape(CH // 8, 8, 128), axis=0)
    return t if acc is None else acc + t


def _stats(chunks):
    s1 = s2 = shift = None
    for c in chunks:
        if shift is None:
            shift = c[0:1]
        d = c - shift
        s1 = _fold(s1, d)
        s2 = _fold(s2, d * d)
    m1 = jnp.sum(s1, axis=0, keepdims=True) * (1.0 / D)
    m2 = jnp.sum(s2, axis=0, keepdims=True) * (1.0 / D)
    var = jnp.maximum(m2 - m1 * m1, 0.0)
    return shift + m1, lax.rsqrt(var + EPS)


def _ln0(v):
    m = _sum0(v) * (1.0 / D)
    c = v - m
    var = _sum0(c * c) * (1.0 / D)
    return c * lax.rsqrt(var + EPS)


def _kernel(x_hbm, wq_hbm, wk_hbm, wv_hbm, wo_hbm, beta_ref, wr_ref, wg_hbm, wu_hbm, wd_hbm,
            out_hbm,
            xbuf, wq_v, wk_v, wv_v, wo_v, wg_v, wu_v, wd_v,
            wall, wo_t, wr_tab,
            k_buf, pk_buf, q_buf, pq_buf, v_buf,
            s0, s1, m0, m1, am_buf, o_buf, gm_tab, g_tab,
            m_st, h_buf, l_buf, obuf,
            sems):
    def x_copy(s):
        return pltpu.make_async_copy(x_hbm.at[0, :, pl.ds(s * L, L)], xbuf.at[s], sems.at[s])
    cp_wk = pltpu.make_async_copy(wk_hbm, wk_v, sems.at[4])
    cp_wq = pltpu.make_async_copy(wq_hbm, wq_v, sems.at[5])
    cp_wv = pltpu.make_async_copy(wv_hbm, wv_v, sems.at[6])
    cp_wo = pltpu.make_async_copy(wo_hbm, wo_v, sems.at[7])
    cp_wg = pltpu.make_async_copy(wg_hbm, wg_v, sems.at[8])
    cp_wu = pltpu.make_async_copy(wu_hbm, wu_v, sems.at[9])
    cp_wd = pltpu.make_async_copy(wd_hbm, wd_v, sems.at[10])

    def o_copy(s):
        return pltpu.make_async_copy(obuf.at[s], out_hbm.at[0, :, pl.ds(s * L, L)], sems.at[11 + s])

    def x0_copy(i):
        return pltpu.make_async_copy(x_hbm.at[0, :, pl.ds(i * 256, 256)], xbuf.at[0, :, pl.ds(i * 256, 256)],
                                     sems.at[16 * i])

    x0_copy(0).start(); cp_wq.start(); x0_copy(1).start()

    gate = jax.nn.sigmoid(beta_ref[...].astype(f32).reshape(1, H))
    rowi = lax.broadcasted_iota(jnp.int32, (640, H), 0)
    coli = lax.broadcasted_iota(jnp.int32, (640, H), 1)
    gcol = jnp.sum(jnp.where((rowi >= coli * DH) & (rowi < coli * DH + DH), gate, 0.0), axis=1, keepdims=True)
    gfull = jnp.broadcast_to(gcol, (640, 128))
    gm_tab[...] = 1.0 - gfull
    g_tab[...] = gfull
    wr_tab[...] = jnp.broadcast_to(wr_ref[...].astype(f32).reshape(1, D), (128, D)).T
    am_buf[...] = jnp.zeros_like(am_buf)
    m_st[...] = jnp.zeros_like(m_st)
    o_buf[...] = jnp.zeros_like(o_buf)
    v_buf[...] = jnp.zeros_like(v_buf)
    pq_buf[...] = jnp.zeros_like(pq_buf)
    pk_buf[...] = jnp.zeros_like(pk_buf)
    k_buf[...] = jnp.zeros_like(k_buf)

    def put_padded(w_ref, base):
        wT = pltpu.bitcast(w_ref[...].T, u32)
        for g in range(G):
            w = min(GW, D - g * GW) // 2
            r0 = (base + GO[g]) // 2
            wall[r0:r0 + w, :] = wT[g * 63:g * 63 + w]
            wall[r0 + w:r0 + GR[g] // 2, :] = jnp.zeros((GR[g] // 2 - w, D), u32)

    row64 = lax.broadcasted_iota(jnp.int32, (64, 128), 0)
    vrow = lax.broadcasted_iota(jnp.int32, (16, 128), 0)
    kk = lax.broadcasted_iota(jnp.int32, (128, 128), 0)
    qq = lax.broadcasted_iota(jnp.int32, (128, 128), 1)
    causal = kk <= qq
    bd = jnp.zeros((128, 128), jnp.bool_)
    for r in range(7):
        bd = bd | ((kk >= r * DH) & (kk < r * DH + DH) & (qq >= r * DH) & (qq < r * DH + DH))
    lane = lax.broadcasted_iota(jnp.int32, (1, 128), 1)
    zr = lax.broadcasted_iota(jnp.int32, (16, 128), 0)
    zc = lax.broadcasted_iota(jnp.int32, (16, 128), 1)
    zmask = (zc >= zr * DH) & (zc < zr * DH + DH)

    def qk(h, s_buf, m_buf):
        g = h // 7
        r = h - g * 7
        qmask = (row64 >= 9 * r) & (row64 < 9 * r + 9)
        for j in reversed(range(NT)):
            n = 128 * (j + 1)
            qt = pltpu.bitcast(jnp.where(qmask, q_buf[g, j], jnp.uint32(0)), bf16)
            kt = pltpu.bitcast(k_buf[g, 0:n // 2, :], bf16)
            s = jnp.dot(kt, qt, preferred_element_type=f32)
            sd = jnp.where(causal, s[n - 128:], -1e30)
            mx = jnp.max(sd.reshape(16, 8, 128), axis=0)
            s_buf[OFF[j] + n - 128:OFF[j] + n, :] = sd
            if j > 0:
                s_buf[OFF[j]:OFF[j] + n - 128, :] = s[:n - 128]
                mx = jnp.maximum(mx, jnp.max(s[:n - 128].reshape(16 * j, 8, 128), axis=0))
            m_buf[j] = mx

    def pv(h, s_buf, m_buf):
        gm = gm_tab[pl.ds(DH * h, 24), :]
        for j in range(NT):
            n = 128 * (j + 1)
            m = jnp.max(m_buf[j], axis=0, keepdims=True)
            p = jnp.exp2(s_buf[OFF[j]:OFF[j] + n, :] - m).astype(bf16)
            vs = []
            for kb in range(j + 1):
                vv = v_buf[kb, pl.ds(9 * h, 16), :]
                vv = jnp.where(vrow == 9, jnp.uint32(ONE_LO), vv)
                vs.append(pltpu.bitcast(vv, bf16))
            va = jnp.concatenate(vs, axis=1) if j > 0 else vs[0]
            o = jnp.dot(va, p, preferred_element_type=f32)
            o = (o[:24] * gm) * (1.0 / o[18:19]) + am_buf[j, pl.ds(DH * h, 24), :]
            o_buf[j, pl.ds(DH * h, 24), :] = o

    def ln_in(s, j):
        ld = lambda c: xbuf[s, c * CH:(c + 1) * CH, j * 128:(j + 1) * 128].astype(f32)
        mean, rstd = _stats(ld(c) for c in range(D // CH))
        return jnp.concatenate([((ld(c) - mean) * rstd).astype(bf16) for c in range(D // CH)], axis=0)

    def proj_q(xn, j):
        t = jnp.dot(pltpu.bitcast(wall[0:NP // 2, :], bf16), xn, preferred_element_type=f32)
        for g in range(G):
            qg = t[GO[g]:GO[g] + GR[g]]
            q_buf[g, j, 0:GR[g] // 2, :] = pltpu.bitcast((qg * QSCALE).astype(bf16), u32)
            pq_buf[g, j, 0:GR[g] // 2, :] = pltpu.bitcast(_phi(qg).astype(bf16), u32)

    def proj_k(xn, j):
        t = jnp.dot(pltpu.bitcast(wall[NP // 2:NP, :], bf16), xn, preferred_element_type=f32)
        for g in range(G):
            kg = t[GO[g]:GO[g] + GR[g]]
            pk_buf[g, j, 0:GR[g] // 2, :] = pltpu.bitcast(_phi(kg).astype(bf16), u32)
            kb = kg.astype(bf16)
            if GR[g] < 128:
                kb = jnp.concatenate([kb, jnp.zeros((128 - GR[g], 128), bf16)], axis=0)
            k_buf[g, 64 * j:64 * (j + 1), :] = pltpu.bitcast(kb.T, u32)

    def proj_v(xn, j):
        t = jnp.dot(pltpu.bitcast(wall[NP:NP + D // 2, :], bf16), xn, preferred_element_type=f32)
        v_buf[j, 0:D // 2, :] = pltpu.bitcast(t.astype(bf16), u32)

    def retrieve():
        r8 = lax.broadcasted_iota(jnp.int32, (8, 128), 0)
        for g in range(G):
            mb = jnp.where(bd, m_st[g, 0:128, :], 0.0).astype(bf16)
            zb = jnp.where(zmask, m_st[g, 128:129, :], 0.0).astype(bf16)
            lhs = jnp.concatenate([mb[:GR[g]], zb], axis=0)
            for j in range(NT):
                rr = jnp.dot(lhs, pltpu.bitcast(pq_buf[g, j], bf16), preferred_element_type=f32)
                rd = 1.0 / (rr[GR[g]:GR[g] + 8] + 1e-6)
                rb = [jnp.broadcast_to(rd[i:i + 1], (8, 128)) for i in range(8)]
                for v in range(GR[g] // 8):
                    h1, h2 = (8 * v) // DH, (8 * v + 7) // DH
                    e = rb[h1] if h1 == h2 else jnp.where(r8 < h2 * DH - 8 * v, rb[h1], rb[h2])
                    gg = g_tab[g * GW + 8 * v:g * GW + 8 * v + 8, :]
                    am_buf[j, g * GW + 8 * v:g * GW + 8 * v + 8, :] = (gg * rr[8 * v:8 * v + 8]) * e

    def update():
        ones = jnp.ones((16, 128), bf16)
        for g in range(G):
            acc = m_st[g]
            for kb in range(NT):
                vg = jnp.concatenate([pltpu.bitcast(v_buf[kb, g * 63:g * 63 + 64, :], bf16), ones], axis=0)
                acc = acc + lax.dot_general(vg, pltpu.bitcast(pk_buf[g, kb], bf16), _NT,
                                            preferred_element_type=f32)
            m_st[g] = acc

    def out_tile(s, j, rbest, ibest):
        att = jnp.dot(pltpu.bitcast(wo_t[...], bf16), o_buf[j, 0:D, :].astype(bf16), preferred_element_type=f32)
        t = s * NT + j

        def resid():
            for c in range(D // CH):
                rows = slice(c * CH, (c + 1) * CH)
                hh = xbuf[s, rows, j * 128:(j + 1) * 128].astype(f32) + att[rows]
                h_buf[t, rows, :] = hh
                yield hh
        mean, rstd = _stats(resid())
        racc = None
        for c in range(D // CH):
            rows = slice(c * CH, (c + 1) * CH)
            hh = h_buf[t, rows, :]
            ln = (hh - mean) * rstd
            obuf[s, rows, j * 128:(j + 1) * 128] = (hh + ln).astype(bf16)
            l_buf[t, rows, :] = ln.astype(bf16)
            racc = _fold(racc, ln * wr_tab[rows, :])
        r = jnp.sum(racc, axis=0, keepdims=True)
        take = r > rbest
        return jnp.where(take, r, rbest), jnp.where(take, lane + (s * L + j * 128), ibest)

    x0_copy(0).wait()
    cp_wq.wait()
    cp_wk.start(); cp_wv.start(); cp_wo.start(); x_copy(1).start()
    xns = [ln_in(0, j) for j in range(2)]
    put_padded(wq_v, 0)
    proj_q(xns[0], 0)
    x0_copy(1).wait()
    xns += [ln_in(0, j) for j in range(2, NT)]
    proj_q(xns[1], 1)
    proj_q(xns[2], 2)
    cp_wk.wait(); cp_wv.wait()
    x_copy(2).start(); x_copy(3).start()
    cp_wg.start(); cp_wu.start(); cp_wd.start()
    proj_q(xns[3], 3)
    put_padded(wk_v, NP)
    wall[NP:NP + D // 2, :] = pltpu.bitcast(wv_v[...].T, u32)
    for j in range(NT):
        proj_k(xns[j], j)
    proj_v(xns[0], 0)
    cp_wo.wait()
    for j in range(1, NT):
        proj_v(xns[j], j)
    wo_t[...] = pltpu.bitcast(wo_v[...].T, u32)
    qk(0, s0, m0)

    def segment(s, carry):
        def heads(i, c):
            for a in range(HU // 2):
                h = i * HU + 2 * a
                qk(h + 1, s1, m1)
                pv(h, s0, m0)
                qk(h + 2, s0, m0)
                pv(h + 1, s1, m1)
            return c
        lax.fori_loop(0, (H - 2) // HU, heads, 0)

        def mid(rbest, ibest):
            x_copy(s + 1).wait()
            qk(H - 1, s1, m1)
            pv(H - 2, s0, m0)
            update()
            xn = ln_in(s + 1, 0)
            proj_q(xn, 0)
            proj_k(xn, 0)
            pv(H - 1, s1, m1)
            proj_v(xn, 0)
            for j in range(NT):
                rbest, ibest = out_tile(s, j, rbest, ibest)
                if j + 1 < NT:
                    xn = ln_in(s + 1, j + 1)
                    proj_q(xn, j + 1)
                    proj_k(xn, j + 1)
                    proj_v(xn, j + 1)
            o_copy(s).start()
            retrieve()
            qk(0, s0, m0)
            return rbest, ibest

        def last(rbest, ibest):
            qk(H - 1, s1, m1)
            pv(H - 2, s0, m0)
            pv(H - 1, s1, m1)
            for j in range(NT):
                rbest, ibest = out_tile(s, j, rbest, ibest)
            o_copy(s).start()
            return rbest, ibest

        return lax.cond(s < NSEG - 1, mid, last, *carry)

    rbest, ibest = lax.fori_loop(
        0, NSEG, segment, (jnp.full((1, 128), -jnp.inf, f32), jnp.zeros((1, 128), jnp.int32)))

    rmax = jnp.max(rbest, axis=1, keepdims=True)
    imin = jnp.min(jnp.where(rbest == rmax, ibest.astype(f32), float(S)), axis=1, keepdims=True).astype(jnp.int32)
    tile = jnp.clip(imin[0, 0] // 128, 0, S // 128 - 1)
    onehot = lane == (imin & 127)
    oh = jnp.broadcast_to(jnp.where(onehot, 1.0, 0.0), (16, 128)).astype(bf16)
    xs = lax.dot_general(oh, l_buf[tile], _NT, preferred_element_type=f32).astype(bf16)
    hh = h_buf[tile]
    ln = _ln0(hh)
    cp_wg.wait(); cp_wu.wait(); cp_wd.wait()
    y = jnp.zeros((D, 128), f32)
    for c in range(F // FCH):
        cs = slice(c * FCH, (c + 1) * FCH)
        gt = jnp.dot(xs, wg_v[:, cs], preferred_element_type=f32)
        up = jnp.dot(xs, wu_v[:, cs], preferred_element_type=f32)
        act = (gt * jax.nn.sigmoid(gt) * up).astype(bf16).astype(f32)[0:1]
        pr = wd_v[:, cs].astype(f32) * act
        for cc in range(FCH // 128):
            y = y + pr[:, cc * 128:(cc + 1) * 128]
    y = jnp.sum(y, axis=1, keepdims=True) * jax.nn.sigmoid(rmax)
    new_tile = jnp.where(onehot, hh + (ln + y), hh + ln).astype(bf16)
    for s in range(NSEG):
        o_copy(s).wait()
    obuf[0, :, 0:128] = new_tile
    fin = pltpu.make_async_copy(obuf.at[0, :, 0:128],
                                out_hbm.at[0, :, pl.ds(pl.multiple_of(tile * 128, 128), 128)], sems.at[15])
    fin.start()
    fin.wait()


@jax.jit
def pallas_sequential_preLN__memory_aug_infini_attn__moe_arch_mod__prompt_kernel(
    A_x: jax.Array,
    A_wq: jax.Array,
    A_wk: jax.Array,
    A_wv: jax.Array,
    A_wo: jax.Array,
    A_beta: jax.Array,
    B_x: jax.Array,
    B_w_r: jax.Array,
    B_w_gate: jax.Array,
    B_w_up: jax.Array,
    B_w_down: jax.Array,
):
    hbm = pl.BlockSpec(memory_space=pltpu.HBM)
    vmem_spec = pl.BlockSpec(memory_space=pltpu.VMEM)
    V = pltpu.VMEM
    scratch = [
        V((NSEG, D, L), bf16),
        V((D, D), bf16), V((D, D), bf16), V((D, D), bf16), V((D, D), bf16),
        V((D, F), bf16), V((D, F), bf16), V((D, F), bf16),
        V((NP + D // 2, D), u32), V((D // 2, D), u32), V((D, 128), f32),
        V((G, L // 2, 128), u32), V((G, NT, 64, 128), u32),
        V((G, NT, 64, 128), u32), V((G, NT, 64, 128), u32),
        V((NT, 320, 128), u32),
        V((1280, 128), f32), V((1280, 128), f32), V((NT, 8, 128), f32), V((NT, 8, 128), f32),
        V((NT, 640, 128), f32), V((NT, 640, 128), f32), V((640, 128), f32), V((640, 128), f32),
        V((G, 144, 128), f32),
        V((S // 128, D, 128), f32), V((S // 128, D, 128), bf16), V((NSEG, D, L), bf16),
        pltpu.SemaphoreType.DMA((17,)),
    ]
    out_t = pl.pallas_call(
        _kernel,
        out_shape=jax.ShapeDtypeStruct((1, D, S), A_x.dtype),
        in_specs=[hbm] * 5 + [vmem_spec, vmem_spec] + [hbm] * 3,
        out_specs=hbm,
        scratch_shapes=scratch,
        compiler_params=pltpu.CompilerParams(vmem_limit_bytes=100 * 1024 * 1024),
    )(jnp.swapaxes(A_x, 1, 2), A_wq, A_wk, A_wv, A_wo, A_beta, B_w_r, B_w_gate, B_w_up, B_w_down.T)
    return jnp.swapaxes(out_t, 1, 2)
```
